```python
import jax
import jax.numpy as jnp

def _softmax(x, axis=-1):
    return jax.nn.softmax(x, axis=axis)

def _gelu(x):
    return jax.nn.gelu(x, approximate=True)

def _silu(x):
    return jax.nn.silu(x)

def _sigmoid(x):
    return jax.nn.sigmoid(x)

def _layernorm(x, axis=-1, eps=1e-05):
    m = jnp.mean(x, axis=axis, keepdims=True)
    v = jnp.var(x, axis=axis, keepdims=True)
    return (x - m) / jnp.sqrt(v + eps)

def _scatter_add(tgt, idx, src, axis=0):
    return tgt.at[idx].add(src)

def _segment_sum(src, seg, n):
    return jax.ops.segment_sum(src, seg, n)

class _Rng:

    def __init__(self, key):
        self._k = key

    def _next(self):
        self._k, sub = jax.random.split(self._k)
        return sub

    def normal(self, shape):
        return jax.random.normal(self._next(), shape, dtype=jnp.bfloat16)

    def randint(self, lo, hi, shape):
        return jax.random.randint(self._next(), shape, lo, hi, dtype=jnp.int32)

    def uniform(self, shape, lo=0.0, hi=1.0):
        return jax.random.uniform(self._next(), shape, jnp.bfloat16, lo, hi)

    def permutation(self, n):
        return jax.random.permutation(self._next(), n)
kernel_name = 'adaLN_cond__gqa_block_cached__moe_arch_mod__prompt'

def setup_inputs():
    _rng = _Rng(jax.random.key(int.from_bytes(__import__("os").urandom(4), "little")))
    _w = lambda a: (lambda t: t.astype(jnp.bfloat16) if jnp.issubdtype(t.dtype, jnp.floating) else t)(jnp.asarray(a))

    def _A_setup():
        B, Sq, D = (1, 2048, 576)
        Hq, Hkv, Sk, Dh = (32, 16, 2048, 128)
        assert Hq % Hkv == 0, (Hq, Hkv)
        return {'x': _w((lambda *s: _rng.normal(s) * 0.05)(B, Sq, D)), 'k_cache': _w((lambda *s: _rng.normal(s) * 0.05)(B, Hkv, Sk, Dh)), 'v_cache': _w((lambda *s: _rng.normal(s) * 0.05)(B, Hkv, Sk, Dh)), 'wq': _w((lambda *s: _rng.normal(s) * 0.05)(D, Hq * Dh) * D ** (-0.5)), 'wo': _w((lambda *s: _rng.normal(s) * 0.05)(Hq * Dh, D) * (Hq * Dh) ** (-0.5))}
    _A_in = _A_setup()

    def _B_setup():
        B, S, D, F, C = (1, 2048, 576, 4608, 8)
        return {'x': _w((lambda *s: _rng.normal(s) * 0.05)(B, S, D)), 'w_r': _w((lambda *s: _rng.normal(s) * 0.05)(D)), 'w_gate': _w((lambda *s: _rng.normal(s) * 0.05)(D, F)), 'w_up': _w((lambda *s: _rng.normal(s) * 0.05)(D, F)), 'w_down': _w((lambda *s: _rng.normal(s) * 0.05)(F, D))}
    _B_in = _B_setup()
    return {'A_x': _A_in['x'], 'A_k_cache': _A_in['k_cache'], 'A_v_cache': _A_in['v_cache'], 'A_wq': _A_in['wq'], 'A_wo': _A_in['wo'], 'B_x': _B_in['x'], 'B_w_r': _B_in['w_r'], 'B_w_gate': _B_in['w_gate'], 'B_w_up': _B_in['w_up'], 'B_w_down': _B_in['w_down'], 'c': _w((lambda *s: _rng.normal(s) * 0.05)(1, 576)), 'w_mod': _w((lambda *s: _rng.normal(s) * 0.05)(576, 6 * 576) * 576 ** (-0.5))}

def reference(A_x, A_k_cache, A_v_cache, A_wq, A_wo, B_x, B_w_r, B_w_gate, B_w_up, B_w_down, c, w_mod):

    def _A_ref(x, k_cache, v_cache, wq, wo):
        B, Sq, D = x.shape
        Hq, Dh = (32, 128)
        Hkv = k_cache.shape[1]
        rep = Hq // Hkv
        q = (lambda x, *d: x.transpose(*d))((x @ wq).reshape(B, Sq, Hq, Dh), 0, 2, 1, 3)
        k = jnp.repeat(k_cache, rep, axis=1)
        v = jnp.repeat(v_cache, rep, axis=1)
        scores = jnp.einsum('bhqd,bhkd->bhqk', q, k) * Dh ** (-0.5)
        p = _softmax(scores, axis=-1)
        o = jnp.einsum('bhqk,bhkd->bhqd', p, v)
        return (lambda x, *d: x.transpose(*d))(o, 0, 2, 1, 3).reshape(B, Sq, Hq * Dh) @ wo

    def _B_ref(x, w_r, w_gate, w_up, w_down):
        B, S, D = x.shape
        C = 8
        r = x @ w_r
        idx = jnp.argsort(-r, axis=-1)[:, :C]
        idx_e = jnp.repeat(idx.reshape(B, C, 1), D, axis=2)
        x_sel = jnp.take_along_axis(x, idx_e, axis=1)
        g = _silu(x_sel @ w_gate)
        u = x_sel @ w_up
        y = g * u @ w_down
        r_sel = _sigmoid(jnp.take_along_axis(r, idx, axis=1))
        y = y * r_sel.reshape(B, C, 1)
        b_off = (jnp.arange(B) * S).reshape(B, 1)
        flat_idx = (idx + b_off).reshape(B * C)
        zero = (x * 0.0).reshape(B * S, D)
        upd = _scatter_add(zero, flat_idx, y.reshape(B * C, D), axis=0)
        return x + upd.reshape(B, S, D)
    x = A_x
    mod = (_silu(c) @ w_mod).reshape(c.shape[0], 6, 1, -1)
    sa, ca, ga, sb, cb, gb = (mod[:, 0].copy(), mod[:, 1].copy(), mod[:, 2].copy(), mod[:, 3].copy(), mod[:, 4].copy(), mod[:, 5].copy())
    h = _layernorm(x, axis=-1) * (1 + ca) + sa
    x = x + ga * _A_ref(h, A_k_cache, A_v_cache, A_wq, A_wo)
    h = _layernorm(x, axis=-1) * (1 + cb) + sb
    x = x + gb * _B_ref(h, B_w_r, B_w_gate, B_w_up, B_w_down)
    return x
```

```python
import contextlib
import math

import jax
import jax.numpy as jnp
from jax import lax
import jax.experimental.pallas as pl
import jax.experimental.pallas.tpu as pltpu

F32 = jnp.float32
BF16 = jnp.bfloat16
U32 = jnp.uint32
NT_DIMS = (((1,), (1,)), ((), ()))

S = 2048
D = 576
HQ = 32
HKV = 16
DH = 128
FF = 4608
TOPC = 8
EPS = 1e-5
BQ = 256
BM = 256
NBM = S // BM
WQ_CHUNKS = ((0, 512), (512, 512), (1024, 1024), (2048, 1024), (3072, 1024))
NWC = len(WQ_CHUNKS)
QSCALE = (DH ** -0.5) * math.log2(math.e)
PROFILE = False


def _scope(name):
  return jax.named_scope(name) if PROFILE else contextlib.nullcontext()


def _rb(x):
  return x.astype(BF16).astype(F32)


def _ln_mod_t(x, scale1, shift):
  inv_d = 1.0 / D
  cen = x - jnp.sum(x, axis=0, keepdims=True) * inv_d
  var = jnp.sum(cen * cen, axis=0, keepdims=True) * inv_d
  return cen * lax.rsqrt(var + EPS) * scale1 + shift


def _rep(a, n):
  return jnp.concatenate([a] * (n // 128), axis=1) if n > 128 else a


def _cols(row):
  return jnp.broadcast_to(row, (128, row.shape[1])).T


def _kernel(xt_hbm, k_hbm, v_hbm, wq_hbm, wot_hbm, wr_hbm, wg_hbm, wu_hbm, wdt_hbm,
            c_hbm, wm_hbm, out_hbm,
            xt_v, q_v, o_v, k_v, v_v, wq_v, wot_v, wr_v, wg_v, wu_v, wdt_v,
            c_v, wm_v, col_v, c0_v, r_v, out_v, idx_s,
            sems, kv_sems, wq_sems, out_sems, patch_sems):

  def cp(src, dst, i):
    return pltpu.make_async_copy(src, dst, sems.at[i])

  c_cp = cp(c_hbm, c_v, 0)
  wm_a_cp = cp(wm_hbm.at[:, pl.ds(0, 2 * D)], wm_v.at[:, pl.ds(0, 2 * D)], 1)
  x_a_cp = cp(xt_hbm.at[0, :, pl.ds(0, 2 * BM)], xt_v.at[:, pl.ds(0, 2 * BM)], 2)
  x_b_cp = cp(xt_hbm.at[0, :, pl.ds(2 * BM, S - 2 * BM)], xt_v.at[:, pl.ds(2 * BM, S - 2 * BM)], 3)
  wm_b_cp = cp(wm_hbm.at[:, pl.ds(2 * D, 4 * D)], wm_v.at[:, pl.ds(2 * D, 4 * D)], 4)
  wo_cp = cp(wot_hbm, wot_v, 5)
  wr_cp = cp(wr_hbm, wr_v, 6)
  wg_cp = cp(wg_hbm, wg_v, 7)
  wu_cp = cp(wu_hbm, wu_v, 8)
  wd_cp = cp(wdt_hbm, wdt_v, 9)
  wq_cps = [pltpu.make_async_copy(wq_hbm.at[:, pl.ds(c0, n)], wq_v.at[:, pl.ds(c0, n)], wq_sems.at[i])
            for i, (c0, n) in enumerate(WQ_CHUNKS)]
  out_cps = [pltpu.make_async_copy(out_v.at[:, pl.ds(i * BM, BM)], out_hbm.at[0, :, pl.ds(i * BM, BM)],
                                   out_sems.at[i]) for i in range(NBM)]

  def kv_cp(g, slot):
    return (pltpu.make_async_copy(k_hbm.at[0, g], k_v.at[slot], kv_sems.at[0, slot]),
            pltpu.make_async_copy(v_hbm.at[0, g], v_v.at[slot], kv_sems.at[1, slot]))

  c_cp.start()
  wm_a_cp.start()
  x_a_cp.start()
  wq_cps[0].start()
  wq_cps[1].start()

  with _scope("prologue"):
    c_cp.wait()
    cf = c_v[...].astype(F32)
    sc = _rb(cf * jax.nn.sigmoid(cf))
    sc16 = jnp.broadcast_to(sc, (16, D)).astype(BF16)
    wm_a_cp.wait()
    mod_a = jnp.dot(sc16, wm_v[:, pl.ds(0, 2 * D)], preferred_element_type=F32)
    mod_a = _cols(_rb(mod_a[0:1, :]))
    sa1 = mod_a[0:D]
    ca11 = _rb(1.0 + mod_a[D:2 * D])

  def ln1(tok0, n):
    ht = _ln_mod_t(xt_v[:, pl.ds(tok0, n)].astype(F32), _rep(ca11, n), _rep(sa1, n))
    return ht.T.astype(BF16)

  def qproj(h, tok0, n, col0, ncol):
    q = jnp.dot(h, wq_v[:, pl.ds(col0, ncol)], preferred_element_type=F32)
    q = (q * QSCALE).astype(BF16)
    for hl in range(ncol // DH):
      q_v[col0 // DH + hl, pl.ds(tok0, n), :] = q[:, hl * DH:(hl + 1) * DH]

  with _scope("qproj"):
    x_a_cp.wait()
    h01 = ln1(0, 2 * BM)
    for ci, d in enumerate(wq_cps):
      d.wait()
      if ci == 0:
        for d2 in wq_cps[2:]:
          d2.start()
        x_b_cp.start()
      if ci == NWC - 1:
        x_b_cp.wait()
        for d2 in kv_cp(0, 0):
          d2.start()
        wm_b_cp.start()
        wr_cp.start()
      qproj(h01, 0, 2 * BM, *WQ_CHUNKS[ci])
    for i in range(2, NBM):
      h = ln1(i * BM, BM)
      qproj(h, i * BM, BM, 0, HQ * DH)

  def group(g, carry):
    slot = g % 2

    @pl.when(g + 1 < HKV)
    def _():
      for d in kv_cp(g + 1, 1 - slot):
        d.start()

    for gi, d in enumerate((wo_cp, wg_cp, wu_cp, wd_cp)):
      @pl.when(g == 2 * gi + 1)
      def _():
        d.start()

    for d in kv_cp(g, slot):
      d.wait()
    k = k_v[slot]
    v = v_v[slot]
    for a in range(HQ // HKV):
      hd = g * (HQ // HKV) + a
      for j in range(S // BQ):
        rows = pl.ds(j * BQ, BQ)
        s = lax.dot_general(q_v[hd, rows, :], k, NT_DIMS, preferred_element_type=F32)
        m = jnp.max(s, axis=1, keepdims=True)
        p = jnp.exp2(s - m)
        l = jnp.sum(p, axis=1, keepdims=True)
        o = jnp.dot(p.astype(BF16), v, preferred_element_type=F32)
        o_v[hd, rows, :] = (o * pltpu.reciprocal(l, approx=True)).astype(BF16)
    return carry

  with _scope("attn"):
    lax.fori_loop(0, HKV, group, 0)

  with _scope("oproj"):
    wo_cp.wait()
    wm_b_cp.wait()
    wr_cp.wait()
    mod_b = jnp.dot(sc16, wm_v[:, pl.ds(2 * D, 4 * D)], preferred_element_type=F32)
    mod_b = _cols(_rb(mod_b[0:1, :]))
    ga1, sb1, cb1, gb1 = mod_b[0:D], mod_b[D:2 * D], _rb(1.0 + mod_b[2 * D:3 * D]), mod_b[3 * D:4 * D]
    wr1 = _cols(wr_v[...].astype(F32).reshape(1, D))
    for t, a in enumerate((ga1, gb1 * cb1, gb1 * sb1, cb1 * wr1, cb1, sb1, gb1, wr1)):
      col_v[t] = a
    c0_v[...] = jnp.broadcast_to(jnp.sum(sb1 * wr1, axis=0, keepdims=True), (8, 128))
    for i in range(NBM):
      rows = pl.ds(i * BM, BM)
      o_cat = jnp.concatenate([o_v[hd, rows, :] for hd in range(HQ)], axis=1)
      att = lax.dot_general(wot_v[...], o_cat, NT_DIMS, preferred_element_type=F32)
      ga, g1, g2, uw = (_rep(col_v[t], BM) for t in range(4))
      x1 = xt_v[:, rows].astype(F32) + ga * att
      x1b = x1.astype(BF16)
      xt_v[:, rows] = x1b
      c0 = x1[0:1, :]
      d0 = x1 - c0
      m0 = jnp.sum(d0, axis=0, keepdims=True) * (1.0 / D)
      var = jnp.sum(d0 * d0, axis=0, keepdims=True) * (1.0 / D) - m0 * m0
      rstd = lax.rsqrt(var + EPS)
      xr = x1b.astype(F32)
      t1 = xr * rstd - (c0 + m0) * rstd
      r = jnp.sum(t1 * uw, axis=0, keepdims=True) + _rep(c0_v[0:1, :], BM)
      out_v[:, rows] = (xr + (g1 * t1 + g2)).astype(BF16)
      r_v[:, rows] = jnp.broadcast_to(_rb(r), (8, BM))

  with _scope("tail"):
    for d in out_cps:
      d.start()

    bits = pltpu.bitcast(r_v[...], jnp.int32)
    hi = lax.shift_right_arithmetic(bits, 16)
    mono = jnp.where(hi < 0, hi ^ 0x7FFF, hi) + 32768
    col = lax.broadcasted_iota(jnp.int32, (8, S), 1)
    key_bits = 0x20000000 | lax.shift_left(mono, 11) | (2047 - col)
    key = pltpu.bitcast(key_bits, F32)
    lane = lax.broadcasted_iota(jnp.int32, (D // 2, 128), 1)
    xsel = jnp.zeros((D // 2, 128), U32)
    for t in range(TOPC):
      best = jnp.max(key, axis=1, keepdims=True)
      key = jnp.where(key == best, 0.0, key)
      bi = 2047 - (pltpu.bitcast(best, jnp.int32) & 2047)
      idx = bi[0, 0]
      idx_s[t] = idx
      tile = pl.ds(pl.multiple_of((idx // 128) * 128, 128), 128)
      shift = (t - idx % 128 + 128) % 128
      xcol = pltpu.roll(pltpu.bitcast(xt_v[:, tile], U32), shift, 1)
      xsel = jnp.where(lane == t, xcol, xsel)

    xt = pltpu.bitcast(xsel, BF16).astype(F32)
    ht = _rb(_ln_mod_t(xt, col_v[4], col_v[5]))
    r_sel = _rb(jnp.sum(ht * col_v[7], axis=0, keepdims=True))
    xsb = ht.T[0:16, :].astype(BF16)
    wg_cp.wait()
    wu_cp.wait()
    wd_cp.wait()
    gate = _rb(jnp.dot(xsb, wg_v[...], preferred_element_type=F32))
    gate = _rb(gate * jax.nn.sigmoid(gate))
    up = _rb(jnp.dot(xsb, wu_v[...], preferred_element_type=F32))
    gu = (gate * up).astype(BF16)
    y = lax.dot_general(gu, wdt_v[...], NT_DIMS, preferred_element_type=F32)
    y128 = jnp.concatenate([y, jnp.zeros((128 - 16, D), F32)], axis=0)
    yt = _rb(y128.T) * _rb(jax.nn.sigmoid(r_sel))
    res = xt + col_v[6] * (ht + yt)
    res_p = pltpu.bitcast(res.astype(BF16), U32)

    for d in out_cps:
      d.wait()

    for t in range(TOPC):
      idx = idx_s[t]
      tile = pl.ds(pl.multiple_of((idx // 128) * 128, 128), 128)
      shift = (idx % 128 - t + 128) % 128
      cur = pltpu.bitcast(out_v[:, tile], U32)
      new = jnp.where(lane == idx % 128, pltpu.roll(res_p, shift, 1), cur)
      out_v[:, tile] = pltpu.bitcast(new, BF16)

    def patch_cp(t):
      tile = pl.ds(pl.multiple_of((idx_s[t] // 128) * 128, 128), 128)
      return pltpu.make_async_copy(out_v.at[:, tile], out_hbm.at[0, :, tile], patch_sems.at[t])

    def first_in_tile(t):
      ok = jnp.bool_(True)
      for t2 in range(t):
        ok = jnp.logical_and(ok, idx_s[t2] // 128 != idx_s[t] // 128)
      return ok

    for t in range(TOPC):
      @pl.when(first_in_tile(t))
      def _():
        patch_cp(t).start()
    for t in range(TOPC):
      @pl.when(first_in_tile(t))
      def _():
        patch_cp(t).wait()


@jax.jit
def pallas_adaLN_cond__gqa_block_cached__moe_arch_mod__prompt_kernel(
    A_x: jax.Array,
    A_k_cache: jax.Array,
    A_v_cache: jax.Array,
    A_wq: jax.Array,
    A_wo: jax.Array,
    B_x: jax.Array,
    B_w_r: jax.Array,
    B_w_gate: jax.Array,
    B_w_up: jax.Array,
    B_w_down: jax.Array,
    c: jax.Array,
    w_mod: jax.Array,
):
  del B_x
  any_spec = pl.BlockSpec(memory_space=pl.ANY)
  vmem = pltpu.VMEM
  scratch = [
      vmem((D, S), BF16),
      vmem((HQ, S, DH), BF16),
      vmem((HQ, S, DH), BF16),
      vmem((2, S, DH), BF16),
      vmem((2, S, DH), BF16),
      vmem((D, HQ * DH), BF16),
      vmem((D, HQ * DH), BF16),
      vmem((D,), BF16),
      vmem((D, FF), BF16),
      vmem((D, FF), BF16),
      vmem((D, FF), BF16),
      vmem((1, D), BF16),
      vmem((D, 6 * D), BF16),
      vmem((8, D, 128), F32),
      vmem((8, 128), F32),
      vmem((8, S), F32),
      vmem((D, S), BF16),
      pltpu.SMEM((TOPC,), jnp.int32),
      pltpu.SemaphoreType.DMA((10,)),
      pltpu.SemaphoreType.DMA((2, 2)),
      pltpu.SemaphoreType.DMA((NWC,)),
      pltpu.SemaphoreType.DMA((NBM,)),
      pltpu.SemaphoreType.DMA((TOPC,)),
  ]
  out_t = pl.pallas_call(
      _kernel,
      in_specs=[any_spec] * 11,
      out_specs=any_spec,
      out_shape=jax.ShapeDtypeStruct((1, D, S), BF16),
      scratch_shapes=scratch,
      compiler_params=pltpu.CompilerParams(vmem_limit_bytes=110 * 1024 * 1024),
      name="adaln_gqa_mod_fused",
  )(jnp.swapaxes(A_x, 1, 2), A_k_cache, A_v_cache, A_wq, A_wo.T, B_w_r, B_w_gate,
    B_w_up, B_w_down.T, c, w_mod)
  return jnp.swapaxes(out_t, 1, 2)
```

```python
import contextlib
import math

import jax
import jax.numpy as jnp
from jax import lax
import jax.experimental.pallas as pl
import jax.experimental.pallas.tpu as pltpu

F32 = jnp.float32
BF16 = jnp.bfloat16
U32 = jnp.uint32
NT_DIMS = (((1,), (1,)), ((), ()))

S = 2048
D = 576
HQ = 32
HKV = 16
DH = 128
FF = 4608
TOPC = 8
EPS = 1e-5
BQ = 256
BM = 256
NBM = S // BM
WQ_CHUNKS = ((0, 512), (512, 768), (1280, 1280), (2560, 1536))
NWC = len(WQ_CHUNKS)
QSCALE = (DH ** -0.5) * math.log2(math.e)
PROFILE = False


def _scope(name):
  return jax.named_scope(name) if PROFILE else contextlib.nullcontext()


def _rb(x):
  return x.astype(BF16).astype(F32)


def _ln_mod_t(x, scale1, shift):
  inv_d = 1.0 / D
  cen = x - jnp.sum(x, axis=0, keepdims=True) * inv_d
  var = jnp.sum(cen * cen, axis=0, keepdims=True) * inv_d
  return cen * lax.rsqrt(var + EPS) * scale1 + shift


def _rep(a, n):
  return jnp.concatenate([a] * (n // 128), axis=1) if n > 128 else a


def _cols(row):
  return jnp.broadcast_to(row, (128, row.shape[1])).T


def _kernel(xt_hbm, k_hbm, v_hbm, wq_hbm, wot_hbm, wr_hbm, wg_hbm, wu_hbm, wdt_hbm,
            c_hbm, wm_hbm, out_hbm,
            xt_v, q_v, o_v, k_v, v_v, wq_v, wot_v, wr_v, wg_v, wu_v, wdt_v,
            c_v, wm_v, modb_v, col_v, st_v, out_v,
            sems, kv_sems, wq_sems, out_sems, patch_sems):

  def cp(src, dst, i):
    return pltpu.make_async_copy(src, dst, sems.at[i])

  c_cp = cp(c_hbm, c_v, 0)
  wm_a_cp = cp(wm_hbm.at[:, pl.ds(0, 2 * D)], wm_v.at[:, pl.ds(0, 2 * D)], 1)
  x_a_cp = cp(xt_hbm.at[0, :, pl.ds(0, 2 * BM)], xt_v.at[:, pl.ds(0, 2 * BM)], 2)
  x_b_cp = cp(xt_hbm.at[0, :, pl.ds(2 * BM, S - 2 * BM)], xt_v.at[:, pl.ds(2 * BM, S - 2 * BM)], 3)
  wm_b_cp = cp(wm_hbm.at[:, pl.ds(2 * D, 4 * D)], wm_v.at[:, pl.ds(2 * D, 4 * D)], 4)
  wo_cp = cp(wot_hbm, wot_v, 5)
  wr_cp = cp(wr_hbm, wr_v, 6)
  wg_cp = cp(wg_hbm, wg_v, 7)
  wu_cp = cp(wu_hbm, wu_v, 8)
  wd_cp = cp(wdt_hbm, wdt_v, 9)
  wq_cps = [pltpu.make_async_copy(wq_hbm.at[:, pl.ds(c0, n)], wq_v.at[:, pl.ds(c0, n)], wq_sems.at[i])
            for i, (c0, n) in enumerate(WQ_CHUNKS)]

  def kv_cp(g, slot):
    return (pltpu.make_async_copy(k_hbm.at[0, g], k_v.at[slot], kv_sems.at[0, slot]),
            pltpu.make_async_copy(v_hbm.at[0, g], v_v.at[slot], kv_sems.at[1, slot]))

  c_cp.start()
  x_a_cp.start()
  wm_a_cp.start()
  wq_cps[0].start()

  def ln_stats(x):
    cen = x - jnp.sum(x, axis=0, keepdims=True) * (1.0 / D)
    var = jnp.sum(cen * cen, axis=0, keepdims=True) * (1.0 / D)
    return cen * lax.rsqrt(var + EPS)

  with _scope("prologue"):
    c_cp.wait()
    cf = c_v[...].astype(F32)
    sc = _rb(cf * jax.nn.sigmoid(cf))
    sc16 = jnp.broadcast_to(sc, (16, D)).astype(BF16)
    x_a_cp.wait()
    xn01 = ln_stats(xt_v[:, pl.ds(0, 2 * BM)].astype(F32))
    wm_a_cp.wait()
    wq_cps[1].start()
    mod_a = jnp.dot(sc16, wm_v[:, pl.ds(0, 2 * D)], preferred_element_type=F32)
    mod_a = _cols(_rb(mod_a[0:1, :]))
    sa1 = mod_a[0:D] * QSCALE
    ca11 = _rb(1.0 + mod_a[D:2 * D]) * QSCALE

  def ln_apply(xn):
    n = xn.shape[1]
    return (xn * _rep(ca11, n) + _rep(sa1, n)).T.astype(BF16)

  def qproj(h, tok0, n, col0, ncol):
    q = jnp.dot(h, wq_v[:, pl.ds(col0, ncol)], preferred_element_type=F32)
    q = q.astype(BF16)
    for hl in range(ncol // DH):
      q_v[col0 // DH + hl, pl.ds(tok0, n), :] = q[:, hl * DH:(hl + 1) * DH]

  with _scope("qproj"):
    h01 = ln_apply(xn01)
    for ci, d in enumerate(wq_cps):
      d.wait()
      if ci + 2 < NWC:
        wq_cps[ci + 2].start()
      if ci == NWC - 3:
        x_b_cp.start()
      if ci == NWC - 1:
        x_b_cp.wait()
        for d2 in kv_cp(0, 0):
          d2.start()
        wm_b_cp.start()
        wr_cp.start()
      qproj(h01, 0, 2 * BM, *WQ_CHUNKS[ci])
    tok0 = 2 * BM
    for n in (512,256,256,256,256):
      h = ln_apply(ln_stats(xt_v[:, pl.ds(tok0, n)].astype(F32)))
      qproj(h, tok0, n, 0, HQ * DH)
      tok0 += n

  def group(g, carry):
    slot = g % 2

    @pl.when(g + 1 < HKV)
    def _():
      for d in kv_cp(g + 1, 1 - slot):
        d.start()

    for gi, d in enumerate((wo_cp, wg_cp, wu_cp, wd_cp)):
      @pl.when(g == 2 * gi + 1)
      def _():
        d.start()

    for d in kv_cp(g, slot):
      d.wait()
    k = k_v[slot]
    v = v_v[slot]
    for a in range(HQ // HKV):
      hd = g * (HQ // HKV) + a
      for j in range(S // BQ):
        rows = pl.ds(j * BQ, BQ)
        s = lax.dot_general(q_v[hd, rows, :], k, NT_DIMS, preferred_element_type=F32)
        m = jnp.max(s, axis=1, keepdims=True)
        p = jnp.exp2(s - m)
        l = jnp.sum(p, axis=1, keepdims=True)
        o = jnp.dot(p.astype(BF16), v, preferred_element_type=F32)
        o_v[hd, rows, :] = (o * pltpu.reciprocal(l, approx=True)).astype(BF16)
    return carry

  with _scope("attn"):
    lax.fori_loop(0, HKV, group, 0)

  with _scope("oproj"):
    wo_cp.wait()
    wm_b_cp.wait()
    wr_cp.wait()
    mod_b = jnp.dot(sc16, wm_v[:, pl.ds(2 * D, 4 * D)], preferred_element_type=F32)
    lane_b = lax.broadcasted_iota(jnp.int32, (1, 4 * D), 1)
    mod_b = _rb(mod_b[0:1, :])
    mod_b = jnp.where((lane_b >= 2 * D) & (lane_b < 3 * D), _rb(1.0 + mod_b), mod_b)
    modb_v[...] = jnp.broadcast_to(mod_b, (8, 4 * D))
    mod_c = _cols(mod_b)
    wr = wr_v[...].astype(F32).reshape(1, D)
    ga1, sb1, cb1, gb1 = mod_c[0:D], mod_c[D:2 * D], mod_c[2 * D:3 * D], mod_c[3 * D:4 * D]
    wr1 = _cols(wr)
    uw1 = cb1 * wr1
    for t, a in enumerate((ga1, uw1, gb1 * cb1, gb1 * sb1)):
      col_v[t] = a
    usum = _rep(jnp.sum(uw1, axis=0, keepdims=True), BM)
    rconst = _rep(jnp.sum(sb1 * wr1, axis=0, keepdims=True), BM)

    for i in range(NBM):
      rows = pl.ds(i * BM, BM)
      o_cat = jnp.concatenate([o_v[hd, rows, :] for hd in range(HQ)], axis=1)
      att = lax.dot_general(wot_v[...], o_cat, NT_DIMS, preferred_element_type=F32)
      x1 = xt_v[:, rows].astype(F32) + _rep(col_v[0], BM) * att
      xt_v[:, rows] = x1.astype(BF16)
      c0 = x1[0:1, :]
      d0 = x1 - c0
      m0 = jnp.sum(d0, axis=0, keepdims=True) * (1.0 / D)
      var = jnp.sum(d0 * d0, axis=0, keepdims=True) * (1.0 / D) - m0 * m0
      rstd = lax.rsqrt(var + EPS)
      r = (jnp.sum(d0 * _rep(col_v[1], BM), axis=0, keepdims=True) - m0 * usum) * rstd + rconst
      st_v[0, :, rows] = jnp.broadcast_to(_rb(r), (8, BM))
      st_v[1, :, rows] = jnp.broadcast_to(rstd, (8, BM))
      st_v[2, :, rows] = jnp.broadcast_to((c0 + m0) * rstd, (8, BM))

  with _scope("tail"):
    wg_cp.wait()
    wu_cp.wait()
    wd_cp.wait()

    def base_out(i, carry):
      rows = pl.ds(pl.multiple_of(i * 128, 128), 128)
      xr = xt_v[:, rows].astype(F32)
      t1 = xr * st_v[1, 0:1, rows] - st_v[2, 0:1, rows]
      out_v[:, rows] = (xr + (col_v[2] * t1 + col_v[3])).astype(BF16)
      pltpu.make_async_copy(out_v.at[:, rows], out_hbm.at[0, :, rows], out_sems.at[0]).start()
      return carry

    lax.fori_loop(0, S // 128, base_out, 0)

    bits = pltpu.bitcast(st_v[0], jnp.int32)
    hi = lax.shift_right_arithmetic(bits, 16)
    mono = jnp.where(hi < 0, hi ^ 0x7FFF, hi) + 32768
    col = lax.broadcasted_iota(jnp.int32, (8, S), 1)
    key_bits = 0x20000000 | lax.shift_left(mono, 11) | (2047 - col)
    key = pltpu.bitcast(key_bits, F32)
    lane = lax.broadcasted_iota(jnp.int32, (D // 2, 128), 1)
    xsel = jnp.zeros((D // 2, 128), U32)
    tiles, lanes = [], []
    for t in range(TOPC):
      best = jnp.max(key, axis=1, keepdims=True)
      key = jnp.where(key == best, 0.0, key)
      bi = 2047 - (pltpu.bitcast(best, jnp.int32) & 2047)
      idx = bi[0, 0]
      tiles.append(lax.shift_right_logical(idx, 7))
      lanes.append(idx & 127)
      tile = pl.ds(pl.multiple_of(tiles[t] * 128, 128), 128)
      xcol = pltpu.roll(pltpu.bitcast(xt_v[:, tile], U32), (t - lanes[t]) & 127, 1)
      xsel = jnp.where(lane == t, xcol, xsel)
    lasts = []
    for t in range(TOPC - 1):
      ok = tiles[t + 1] != tiles[t]
      for t2 in range(t + 2, TOPC):
        ok = jnp.logical_and(ok, tiles[t2] != tiles[t])
      lasts.append(ok)

    xs = pltpu.bitcast(xsel, BF16).astype(F32).T[0:8, :]
    modb = modb_v[...]
    sb, cb, gb = modb[:, D:2 * D], modb[:, 2 * D:3 * D], modb[:, 3 * D:4 * D]
    cen = xs - jnp.sum(xs, axis=1, keepdims=True) * (1.0 / D)
    var = jnp.sum(cen * cen, axis=1, keepdims=True) * (1.0 / D)
    hs = _rb(cen * lax.rsqrt(var + EPS) * cb + sb)
    r_sel = _rb(jnp.sum(hs * wr, axis=1, keepdims=True))
    xsb = jnp.concatenate([hs, jnp.zeros((8, D), F32)], axis=0).astype(BF16)
    gate = _rb(jnp.dot(xsb, wg_v[...], preferred_element_type=F32))
    gate = _rb(gate * jax.nn.sigmoid(gate))
    up = _rb(jnp.dot(xsb, wu_v[...], preferred_element_type=F32))
    gu = (gate * up).astype(BF16)
    y = lax.dot_general(gu, wdt_v[...], NT_DIMS, preferred_element_type=F32)[0:8, :]
    y = _rb(y) * _rb(jax.nn.sigmoid(r_sel))
    res = xs + gb * (hs + y)
    res = jnp.concatenate([res, jnp.zeros((128 - 8, D), F32)], axis=0).T
    res_p = pltpu.bitcast(res.astype(BF16), U32)

    pltpu.make_async_copy(out_v, out_hbm.at[0], out_sems.at[0]).wait()

    def patch_cp(t):
      tile = pl.ds(pl.multiple_of(tiles[t] * 128, 128), 128)
      return pltpu.make_async_copy(out_v.at[:, tile], out_hbm.at[0, :, tile], patch_sems.at[t])

    for t in range(TOPC):
      tile = pl.ds(pl.multiple_of(tiles[t] * 128, 128), 128)
      cur = pltpu.bitcast(out_v[:, tile], U32)
      new = jnp.where(lane == lanes[t], pltpu.roll(res_p, (lanes[t] - t) & 127, 1), cur)
      out_v[:, tile] = pltpu.bitcast(new, BF16)
      if t == TOPC - 1:
        patch_cp(t).start()
      else:
        pl.when(lasts[t])(lambda t=t: patch_cp(t).start())
    for t in range(TOPC - 1):
      pl.when(lasts[t])(lambda t=t: patch_cp(t).wait())
    patch_cp(TOPC - 1).wait()


@jax.jit
def pallas_adaLN_cond__gqa_block_cached__moe_arch_mod__prompt_kernel(
    A_x: jax.Array,
    A_k_cache: jax.Array,
    A_v_cache: jax.Array,
    A_wq: jax.Array,
    A_wo: jax.Array,
    B_x: jax.Array,
    B_w_r: jax.Array,
    B_w_gate: jax.Array,
    B_w_up: jax.Array,
    B_w_down: jax.Array,
    c: jax.Array,
    w_mod: jax.Array,
):
  del B_x
  any_spec = pl.BlockSpec(memory_space=pl.ANY)
  vmem = pltpu.VMEM
  scratch = [
      vmem((D, S), BF16),
      vmem((HQ, S, DH), BF16),
      vmem((HQ, S, DH), BF16),
      vmem((2, S, DH), BF16),
      vmem((2, S, DH), BF16),
      vmem((D, HQ * DH), BF16),
      vmem((D, HQ * DH), BF16),
      vmem((D,), BF16),
      vmem((D, FF), BF16),
      vmem((D, FF), BF16),
      vmem((D, FF), BF16),
      vmem((1, D), BF16),
      vmem((D, 6 * D), BF16),
      vmem((8, 4 * D), F32),
      vmem((4, D, 128), F32),
      vmem((3, 8, S), F32),
      vmem((D, S), BF16),
      pltpu.SemaphoreType.DMA((10,)),
      pltpu.SemaphoreType.DMA((2, 2)),
      pltpu.SemaphoreType.DMA((NWC,)),
      pltpu.SemaphoreType.DMA((1,)),
      pltpu.SemaphoreType.DMA((TOPC,)),
  ]
  out_t = pl.pallas_call(
      _kernel,
      in_specs=[any_spec] * 11,
      out_specs=any_spec,
      out_shape=jax.ShapeDtypeStruct((1, D, S), BF16),
      scratch_shapes=scratch,
      compiler_params=pltpu.CompilerParams(vmem_limit_bytes=110 * 1024 * 1024),
      name="adaln_gqa_mod_fused",
  )(jnp.swapaxes(A_x, 1, 2), A_k_cache, A_v_cache, A_wq, A_wo.T, B_w_r, B_w_gate,
    B_w_up, B_w_down.T, c, w_mod)
  return jnp.swapaxes(out_t, 1, 2)
```

```python
import contextlib
import math

import jax
import jax.numpy as jnp
from jax import lax
import jax.experimental.pallas as pl
import jax.experimental.pallas.tpu as pltpu

F32 = jnp.float32
BF16 = jnp.bfloat16
U32 = jnp.uint32
NT_DIMS = (((1,), (1,)), ((), ()))

S = 2048
D = 576
HQ = 32
HKV = 16
DH = 128
FF = 4608
TOPC = 8
EPS = 1e-5
BQ = 256
BM = 256
NBM = S // BM
WQ_CHUNKS = ((0, 512), (512, 768), (1280, 1280), (2560, 1536))
NWC = len(WQ_CHUNKS)
QSCALE = (DH ** -0.5) * math.log2(math.e)
PROFILE = False


def _scope(name):
  return jax.named_scope(name) if PROFILE else contextlib.nullcontext()


def _rb(x):
  return x.astype(BF16).astype(F32)


def _ln_mod_t(x, scale1, shift):
  inv_d = 1.0 / D
  cen = x - jnp.sum(x, axis=0, keepdims=True) * inv_d
  var = jnp.sum(cen * cen, axis=0, keepdims=True) * inv_d
  return cen * lax.rsqrt(var + EPS) * scale1 + shift


def _rep(a, n):
  return jnp.concatenate([a] * (n // 128), axis=1) if n > 128 else a


def _cols(row):
  return jnp.broadcast_to(row, (128, row.shape[1])).T


def _kernel(xt_hbm, k_hbm, v_hbm, wq_hbm, wot_hbm, wr_hbm, wg_hbm, wu_hbm, wdt_hbm,
            c_hbm, wm_hbm, out_hbm,
            xt_v, q_v, o_v, k_v, v_v, wq_v, wot_v, wr_v, wg_v, wu_v, wdt_v,
            c_v, wm_v, modb_v, col_v, st_v, out_v,
            sems, kv_sems, wq_sems, out_sems, patch_sems):

  def cp(src, dst, i):
    return pltpu.make_async_copy(src, dst, sems.at[i])

  c_cp = cp(c_hbm, c_v, 0)
  wm_a_cp = cp(wm_hbm.at[:, pl.ds(0, 2 * D)], wm_v.at[:, pl.ds(0, 2 * D)], 1)
  x_a_cp = cp(xt_hbm.at[0, :, pl.ds(0, 2 * BM)], xt_v.at[:, pl.ds(0, 2 * BM)], 2)
  x_b_cp = cp(xt_hbm.at[0, :, pl.ds(2 * BM, S - 2 * BM)], xt_v.at[:, pl.ds(2 * BM, S - 2 * BM)], 3)
  wm_b_cp = cp(wm_hbm.at[:, pl.ds(2 * D, 4 * D)], wm_v.at[:, pl.ds(2 * D, 4 * D)], 4)
  wo_cp = cp(wot_hbm, wot_v, 5)
  wr_cp = cp(wr_hbm, wr_v, 6)
  wg_cp = cp(wg_hbm, wg_v, 7)
  wu_cp = cp(wu_hbm, wu_v, 8)
  wd_cp = cp(wdt_hbm, wdt_v, 9)
  wq_cps = [pltpu.make_async_copy(wq_hbm.at[:, pl.ds(c0, n)], wq_v.at[:, pl.ds(c0, n)], wq_sems.at[i])
            for i, (c0, n) in enumerate(WQ_CHUNKS)]

  def kv_cp(g, slot):
    return (pltpu.make_async_copy(k_hbm.at[0, g], k_v.at[slot], kv_sems.at[0, slot]),
            pltpu.make_async_copy(v_hbm.at[0, g], v_v.at[slot], kv_sems.at[1, slot]))

  c_cp.start()
  x_a_cp.start()
  wm_a_cp.start()
  wq_cps[0].start()

  def ln_stats(x):
    cen = x - jnp.sum(x, axis=0, keepdims=True) * (1.0 / D)
    var = jnp.sum(cen * cen, axis=0, keepdims=True) * (1.0 / D)
    return cen * lax.rsqrt(var + EPS)

  with _scope("prologue"):
    c_cp.wait()
    cf = c_v[...].astype(F32)
    sc = _rb(cf * jax.nn.sigmoid(cf))
    sc16 = jnp.broadcast_to(sc, (16, D)).astype(BF16)
    x_a_cp.wait()
    xn01 = ln_stats(xt_v[:, pl.ds(0, 2 * BM)].astype(F32))
    wm_a_cp.wait()
    wq_cps[1].start()
    mod_a = jnp.dot(sc16, wm_v[:, pl.ds(0, 2 * D)], preferred_element_type=F32)
    mod_a = _cols(_rb(mod_a[0:1, :]))
    sa1 = mod_a[0:D] * QSCALE
    ca11 = _rb(1.0 + mod_a[D:2 * D]) * QSCALE

  def ln_apply(xn):
    n = xn.shape[1]
    return (xn * _rep(ca11, n) + _rep(sa1, n)).T.astype(BF16)

  def qproj(h, tok0, n, col0, ncol):
    q = jnp.dot(h, wq_v[:, pl.ds(col0, ncol)], preferred_element_type=F32)
    q = q.astype(BF16)
    for hl in range(ncol // DH):
      q_v[col0 // DH + hl, pl.ds(tok0, n), :] = q[:, hl * DH:(hl + 1) * DH]

  with _scope("qproj"):
    h01 = ln_apply(xn01)
    for ci, d in enumerate(wq_cps):
      d.wait()
      if ci + 2 < NWC:
        wq_cps[ci + 2].start()
      if ci == NWC - 3:
        x_b_cp.start()
      if ci == NWC - 1:
        x_b_cp.wait()
        for d2 in kv_cp(0, 0):
          d2.start()
        for d2 in (wm_b_cp, wr_cp, wo_cp, wg_cp, wu_cp, wd_cp):
          d2.start()
      qproj(h01, 0, 2 * BM, *WQ_CHUNKS[ci])
    tok0 = 2 * BM
    for n in (512,256,256,256,256):
      h = ln_apply(ln_stats(xt_v[:, pl.ds(tok0, n)].astype(F32)))
      qproj(h, tok0, n, 0, HQ * DH)
      tok0 += n

  def group(g, carry):
    slot = g % 2
    nxt = kv_cp(jnp.minimum(g + 1, HKV - 1), 1 - slot)
    k = k_v[slot]
    v = v_v[slot]
    for a in range(HQ // HKV):
      hd = g * (HQ // HKV) + a
      for j in range(S // BQ):
        rows = pl.ds(j * BQ, BQ)
        s = lax.dot_general(q_v[hd, rows, :], k, NT_DIMS, preferred_element_type=F32)
        m = jnp.max(s, axis=1, keepdims=True)
        p = jnp.exp2(s - m)
        l = jnp.sum(p, axis=1, keepdims=True)
        o = jnp.dot(p.astype(BF16), v, preferred_element_type=F32)
        o_v[hd, rows, :] = (o * pltpu.reciprocal(l, approx=True)).astype(BF16)
        if a == 0 and j == 0:
          for d in nxt:
            d.start()
    for d in nxt:
      d.wait()
    return carry

  with _scope("attn"):
    for d in kv_cp(0, 0):
      d.wait()
    lax.fori_loop(0, HKV, group, 0)

  with _scope("oproj"):
    wo_cp.wait()
    wm_b_cp.wait()
    wr_cp.wait()
    mod_b = jnp.dot(sc16, wm_v[:, pl.ds(2 * D, 4 * D)], preferred_element_type=F32)
    lane_b = lax.broadcasted_iota(jnp.int32, (1, 4 * D), 1)
    mod_b = _rb(mod_b[0:1, :])
    mod_b = jnp.where((lane_b >= 2 * D) & (lane_b < 3 * D), _rb(1.0 + mod_b), mod_b)
    modb_v[...] = jnp.broadcast_to(mod_b, (8, 4 * D))
    mod_c = _cols(mod_b)
    wr = wr_v[...].astype(F32).reshape(1, D)
    ga1, sb1, cb1, gb1 = mod_c[0:D], mod_c[D:2 * D], mod_c[2 * D:3 * D], mod_c[3 * D:4 * D]
    wr1 = _cols(wr)
    uw1 = cb1 * wr1
    for t, a in enumerate((ga1, uw1, gb1 * cb1, gb1 * sb1)):
      col_v[t] = a
    usum = _rep(jnp.sum(uw1, axis=0, keepdims=True), BM)
    rconst = _rep(jnp.sum(sb1 * wr1, axis=0, keepdims=True), BM)

    for i in range(NBM):
      rows = pl.ds(i * BM, BM)
      o_cat = jnp.concatenate([o_v[hd, rows, :] for hd in range(HQ)], axis=1)
      att = lax.dot_general(wot_v[...], o_cat, NT_DIMS, preferred_element_type=F32)
      x1 = xt_v[:, rows].astype(F32) + _rep(col_v[0], BM) * att
      xt_v[:, rows] = x1.astype(BF16)
      c0 = x1[0:1, :]
      d0 = x1 - c0
      m0 = jnp.sum(d0, axis=0, keepdims=True) * (1.0 / D)
      var = jnp.sum(d0 * d0, axis=0, keepdims=True) * (1.0 / D) - m0 * m0
      rstd = lax.rsqrt(var + EPS)
      r = (jnp.sum(d0 * _rep(col_v[1], BM), axis=0, keepdims=True) - m0 * usum) * rstd + rconst
      st_v[0, :, rows] = jnp.broadcast_to(_rb(r), (8, BM))
      st_v[1, :, rows] = jnp.broadcast_to(rstd, (8, BM))
      st_v[2, :, rows] = jnp.broadcast_to((c0 + m0) * rstd, (8, BM))

  with _scope("tail"):
    wg_cp.wait()
    wu_cp.wait()
    wd_cp.wait()

    def base_out(i, carry):
      rows = pl.ds(pl.multiple_of(i * 128, 128), 128)
      xr = xt_v[:, rows].astype(F32)
      t1 = xr * st_v[1, 0:1, rows] - st_v[2, 0:1, rows]
      out_v[:, rows] = (xr + (col_v[2] * t1 + col_v[3])).astype(BF16)
      pltpu.make_async_copy(out_v.at[:, rows], out_hbm.at[0, :, rows], out_sems.at[0]).start()
      return carry

    lax.fori_loop(0, S // 128, base_out, 0)

    bits = pltpu.bitcast(st_v[0], jnp.int32)
    hi = lax.shift_right_arithmetic(bits, 16)
    mono = jnp.where(hi < 0, hi ^ 0x7FFF, hi) + 32768
    col = lax.broadcasted_iota(jnp.int32, (8, S), 1)
    key_bits = 0x20000000 | lax.shift_left(mono, 11) | (2047 - col)
    key = pltpu.bitcast(key_bits, F32)
    lane = lax.broadcasted_iota(jnp.int32, (D // 2, 128), 1)
    xsel = jnp.zeros((D // 2, 128), U32)
    tiles, lanes = [], []
    for t in range(TOPC):
      best = jnp.max(key, axis=1, keepdims=True)
      key = jnp.where(key == best, 0.0, key)
      bi = 2047 - (pltpu.bitcast(best, jnp.int32) & 2047)
      idx = bi[0, 0]
      tiles.append(lax.shift_right_logical(idx, 7))
      lanes.append(idx & 127)
      tile = pl.ds(pl.multiple_of(tiles[t] * 128, 128), 128)
      xcol = pltpu.roll(pltpu.bitcast(xt_v[:, tile], U32), (t - lanes[t]) & 127, 1)
      xsel = jnp.where(lane == t, xcol, xsel)
    lasts = []
    for t in range(TOPC - 1):
      ok = tiles[t + 1] != tiles[t]
      for t2 in range(t + 2, TOPC):
        ok = jnp.logical_and(ok, tiles[t2] != tiles[t])
      lasts.append(ok)

    xs = pltpu.bitcast(xsel, BF16).astype(F32).T[0:8, :]
    modb = modb_v[...]
    sb, cb, gb = modb[:, D:2 * D], modb[:, 2 * D:3 * D], modb[:, 3 * D:4 * D]
    cen = xs - jnp.sum(xs, axis=1, keepdims=True) * (1.0 / D)
    var = jnp.sum(cen * cen, axis=1, keepdims=True) * (1.0 / D)
    hs = _rb(cen * lax.rsqrt(var + EPS) * cb + sb)
    r_sel = _rb(jnp.sum(hs * wr, axis=1, keepdims=True))
    xsb = jnp.concatenate([hs, jnp.zeros((8, D), F32)], axis=0).astype(BF16)
    gate = _rb(jnp.dot(xsb, wg_v[...], preferred_element_type=F32))
    gate = _rb(gate * jax.nn.sigmoid(gate))
    up = _rb(jnp.dot(xsb, wu_v[...], preferred_element_type=F32))
    gu = (gate * up).astype(BF16)
    wd = pltpu.bitcast(pltpu.bitcast(wdt_v[...].T, U32), BF16)
    y = jnp.dot(gu, wd, preferred_element_type=F32)[0:8, :]
    y = _rb(y) * _rb(jax.nn.sigmoid(r_sel))
    res = xs + gb * (hs + y)
    res = jnp.concatenate([res, jnp.zeros((128 - 8, D), F32)], axis=0).T
    res_p = pltpu.bitcast(res.astype(BF16), U32)

    pltpu.make_async_copy(out_v, out_hbm.at[0], out_sems.at[0]).wait()

    def patch_cp(t):
      tile = pl.ds(pl.multiple_of(tiles[t] * 128, 128), 128)
      return pltpu.make_async_copy(out_v.at[:, tile], out_hbm.at[0, :, tile], patch_sems.at[t])

    for t in range(TOPC):
      tile = pl.ds(pl.multiple_of(tiles[t] * 128, 128), 128)
      cur = pltpu.bitcast(out_v[:, tile], U32)
      new = jnp.where(lane == lanes[t], pltpu.roll(res_p, (lanes[t] - t) & 127, 1), cur)
      out_v[:, tile] = pltpu.bitcast(new, BF16)
      if t == TOPC - 1:
        patch_cp(t).start()
      else:
        pl.when(lasts[t])(lambda t=t: patch_cp(t).start())
    for t in range(TOPC - 1):
      pl.when(lasts[t])(lambda t=t: patch_cp(t).wait())
    patch_cp(TOPC - 1).wait()


@jax.jit
def pallas_adaLN_cond__gqa_block_cached__moe_arch_mod__prompt_kernel(
    A_x: jax.Array,
    A_k_cache: jax.Array,
    A_v_cache: jax.Array,
    A_wq: jax.Array,
    A_wo: jax.Array,
    B_x: jax.Array,
    B_w_r: jax.Array,
    B_w_gate: jax.Array,
    B_w_up: jax.Array,
    B_w_down: jax.Array,
    c: jax.Array,
    w_mod: jax.Array,
):
  del B_x
  any_spec = pl.BlockSpec(memory_space=pl.ANY)
  vmem = pltpu.VMEM
  scratch = [
      vmem((D, S), BF16),
      vmem((HQ, S, DH), BF16),
      vmem((HQ, S, DH), BF16),
      vmem((2, S, DH), BF16),
      vmem((2, S, DH), BF16),
      vmem((D, HQ * DH), BF16),
      vmem((D, HQ * DH), BF16),
      vmem((D,), BF16),
      vmem((D, FF), BF16),
      vmem((D, FF), BF16),
      vmem((D, FF), BF16),
      vmem((1, D), BF16),
      vmem((D, 6 * D), BF16),
      vmem((8, 4 * D), F32),
      vmem((4, D, 128), F32),
      vmem((3, 8, S), F32),
      vmem((D, S), BF16),
      pltpu.SemaphoreType.DMA((10,)),
      pltpu.SemaphoreType.DMA((2, 2)),
      pltpu.SemaphoreType.DMA((NWC,)),
      pltpu.SemaphoreType.DMA((1,)),
      pltpu.SemaphoreType.DMA((TOPC,)),
  ]
  out_t = pl.pallas_call(
      _kernel,
      in_specs=[any_spec] * 11,
      out_specs=any_spec,
      out_shape=jax.ShapeDtypeStruct((1, D, S), BF16),
      scratch_shapes=scratch,
      compiler_params=pltpu.CompilerParams(vmem_limit_bytes=110 * 1024 * 1024),
      name="adaln_gqa_mod_fused",
  )(jnp.swapaxes(A_x, 1, 2), A_k_cache, A_v_cache, A_wq, A_wo.T, B_w_r, B_w_gate,
    B_w_up, B_w_down.T, c, w_mod)
  return jnp.swapaxes(out_t, 1, 2)
```

```python
import contextlib
import math

import jax
import jax.numpy as jnp
from jax import lax
import jax.experimental.pallas as pl
import jax.experimental.pallas.tpu as pltpu

F32 = jnp.float32
BF16 = jnp.bfloat16
U32 = jnp.uint32
NT_DIMS = (((1,), (1,)), ((), ()))

S = 2048
D = 576
HQ = 32
HKV = 16
DH = 128
FF = 4608
TOPC = 8
EPS = 1e-5
Q_BLOCKS = ((512, 512, 512, 512), (512, 512, 384, 384, 256))
BM = 256
NBM = S // BM
WQ_CHUNKS = ((0, 512), (512, 768), (1280, 1280), (2560, 1536))
NWC = len(WQ_CHUNKS)
QSCALE = (DH ** -0.5) * math.log2(math.e)
PROFILE = False


def _scope(name):
  return jax.named_scope(name) if PROFILE else contextlib.nullcontext()


def _rb(x):
  return x.astype(BF16).astype(F32)


def _ln_mod_t(x, scale1, shift):
  inv_d = 1.0 / D
  cen = x - jnp.sum(x, axis=0, keepdims=True) * inv_d
  var = jnp.sum(cen * cen, axis=0, keepdims=True) * inv_d
  return cen * lax.rsqrt(var + EPS) * scale1 + shift


def _rep(a, n):
  return jnp.concatenate([a] * (n // 128), axis=1) if n > 128 else a


def _cols(row):
  return jnp.broadcast_to(row, (128, row.shape[1])).T


def _kernel(xt_hbm, k_hbm, v_hbm, wq_hbm, wot_hbm, wr_hbm, wg_hbm, wu_hbm, wdt_hbm,
            c_hbm, wm_hbm, out_hbm,
            xt_v, q_v, o_v, k_v, v_v, wq_v, wot_v, wr_v, wg_v, wu_v, wdt_v,
            c_v, wm_v, modb_v, col_v, st_v, out_v,
            sems, kv_sems, wq_sems, out_sems, patch_sems):

  def cp(src, dst, i):
    return pltpu.make_async_copy(src, dst, sems.at[i])

  c_cp = cp(c_hbm, c_v, 0)
  wm_a_cp = cp(wm_hbm.at[:, pl.ds(0, 2 * D)], wm_v.at[:, pl.ds(0, 2 * D)], 1)
  x_a_cp = cp(xt_hbm.at[0, :, pl.ds(0, 2 * BM)], xt_v.at[:, pl.ds(0, 2 * BM)], 2)
  x_b_cp = cp(xt_hbm.at[0, :, pl.ds(2 * BM, S - 2 * BM)], xt_v.at[:, pl.ds(2 * BM, S - 2 * BM)], 3)
  wm_b_cp = cp(wm_hbm.at[:, pl.ds(2 * D, 4 * D)], wm_v.at[:, pl.ds(2 * D, 4 * D)], 4)
  wo_cp = cp(wot_hbm, wot_v, 5)
  wr_cp = cp(wr_hbm, wr_v, 6)
  wg_cp = cp(wg_hbm, wg_v, 7)
  wu_cp = cp(wu_hbm, wu_v, 8)
  wd_cp = cp(wdt_hbm, wdt_v, 9)
  wq_cps = [pltpu.make_async_copy(wq_hbm.at[:, pl.ds(c0, n)], wq_v.at[:, pl.ds(c0, n)], wq_sems.at[i])
            for i, (c0, n) in enumerate(WQ_CHUNKS)]

  def kv_cp(g, slot):
    return (pltpu.make_async_copy(k_hbm.at[0, g], k_v.at[slot], kv_sems.at[0, slot]),
            pltpu.make_async_copy(v_hbm.at[0, g], v_v.at[slot], kv_sems.at[1, slot]))

  c_cp.start()
  x_a_cp.start()
  wm_a_cp.start()
  wq_cps[0].start()

  def ln_stats(x):
    cen = x - jnp.sum(x, axis=0, keepdims=True) * (1.0 / D)
    var = jnp.sum(cen * cen, axis=0, keepdims=True) * (1.0 / D)
    return cen * lax.rsqrt(var + EPS)

  with _scope("prologue"):
    c_cp.wait()
    cf = c_v[...].astype(F32)
    sc = _rb(cf * jax.nn.sigmoid(cf))
    sc16 = jnp.broadcast_to(sc, (16, D)).astype(BF16)
    x_a_cp.wait()
    xn01 = ln_stats(xt_v[:, pl.ds(0, 2 * BM)].astype(F32))
    wm_a_cp.wait()
    wq_cps[1].start()
    mod_a = jnp.dot(sc16, wm_v[:, pl.ds(0, 2 * D)], preferred_element_type=F32)
    mod_a = _cols(_rb(mod_a[0:1, :]))
    sa1 = mod_a[0:D] * QSCALE
    ca11 = _rb(1.0 + mod_a[D:2 * D]) * QSCALE

  def ln_apply(xn):
    n = xn.shape[1]
    return (xn * _rep(ca11, n) + _rep(sa1, n)).T.astype(BF16)

  def qproj(h, tok0, n, col0, ncol):
    q = jnp.dot(h, wq_v[:, pl.ds(col0, ncol)], preferred_element_type=F32)
    q = q.astype(BF16)
    for hl in range(ncol // DH):
      q_v[col0 // DH + hl, pl.ds(tok0, n), :] = q[:, hl * DH:(hl + 1) * DH]

  with _scope("qproj"):
    h01 = ln_apply(xn01)
    for ci, d in enumerate(wq_cps):
      d.wait()
      if ci + 2 < NWC:
        wq_cps[ci + 2].start()
      if ci == NWC - 3:
        x_b_cp.start()
      if ci == NWC - 1:
        x_b_cp.wait()
        for d2 in kv_cp(0, 0):
          d2.start()
        for d2 in (wm_b_cp, wr_cp, wo_cp, wg_cp, wu_cp, wd_cp):
          d2.start()
      qproj(h01, 0, 2 * BM, *WQ_CHUNKS[ci])
    tok0 = 2 * BM
    for n in (512,256,256,256,256):
      h = ln_apply(ln_stats(xt_v[:, pl.ds(tok0, n)].astype(F32)))
      qproj(h, tok0, n, 0, HQ * DH)
      tok0 += n

  def group(g, carry):
    slot = g % 2
    nxt = kv_cp(jnp.minimum(g + 1, HKV - 1), 1 - slot)
    k = k_v[slot]
    v = v_v[slot]
    for a, blocks in enumerate(Q_BLOCKS):
      hd = g * (HQ // HKV) + a
      row0 = 0
      for bq in blocks:
        rows = pl.ds(row0, bq)
        s = lax.dot_general(q_v[hd, rows, :], k, NT_DIMS, preferred_element_type=F32)
        m = jnp.max(s, axis=1, keepdims=True)
        p = jnp.exp2(s - m).astype(BF16)
        l = jnp.sum(p.astype(F32), axis=1, keepdims=True)
        o = jnp.dot(p, v, preferred_element_type=F32)
        o_v[hd, rows, :] = (o * pltpu.reciprocal(l, approx=True)).astype(BF16)
        if a == 0 and row0 == 0:
          for d in nxt:
            d.start()
        row0 += bq
    for d in nxt:
      d.wait()
    return carry

  with _scope("attn"):
    for d in kv_cp(0, 0):
      d.wait()
    lax.fori_loop(0, HKV, group, 0)

  with _scope("oproj"):
    wo_cp.wait()
    wm_b_cp.wait()
    wr_cp.wait()
    mod_b = jnp.dot(sc16, wm_v[:, pl.ds(2 * D, 4 * D)], preferred_element_type=F32)
    lane_b = lax.broadcasted_iota(jnp.int32, (1, 4 * D), 1)
    mod_b = _rb(mod_b[0:1, :])
    mod_b = jnp.where((lane_b >= 2 * D) & (lane_b < 3 * D), _rb(1.0 + mod_b), mod_b)
    modb_v[...] = jnp.broadcast_to(mod_b, (8, 4 * D))
    mod_c = _cols(mod_b)
    wr = wr_v[...].astype(F32).reshape(1, D)
    ga1, sb1, cb1, gb1 = mod_c[0:D], mod_c[D:2 * D], mod_c[2 * D:3 * D], mod_c[3 * D:4 * D]
    wr1 = _cols(wr)
    uw1 = cb1 * wr1
    for t, a in enumerate((ga1, uw1, gb1 * cb1, gb1 * sb1)):
      col_v[t] = a
    usum = _rep(jnp.sum(uw1, axis=0, keepdims=True), BM)
    rconst = _rep(jnp.sum(sb1 * wr1, axis=0, keepdims=True), BM)

    for i in range(NBM):
      rows = pl.ds(i * BM, BM)
      o_cat = jnp.concatenate([o_v[hd, rows, :] for hd in range(HQ)], axis=1)
      att = lax.dot_general(wot_v[...], o_cat, NT_DIMS, preferred_element_type=F32)
      x1 = xt_v[:, rows].astype(F32) + _rep(col_v[0], BM) * att
      xt_v[:, rows] = x1.astype(BF16)
      c0 = x1[0:1, :]
      d0 = x1 - c0
      m0 = jnp.sum(d0, axis=0, keepdims=True) * (1.0 / D)
      var = jnp.sum(d0 * d0, axis=0, keepdims=True) * (1.0 / D) - m0 * m0
      rstd = lax.rsqrt(var + EPS)
      r = (jnp.sum(d0 * _rep(col_v[1], BM), axis=0, keepdims=True) - m0 * usum) * rstd + rconst
      st_v[0, :, rows] = jnp.broadcast_to(_rb(r), (8, BM))
      st_v[1, :, rows] = jnp.broadcast_to(rstd, (8, BM))
      st_v[2, :, rows] = jnp.broadcast_to((c0 + m0) * rstd, (8, BM))

  with _scope("tail"):
    wg_cp.wait()
    wu_cp.wait()
    wd_cp.wait()

    def base_out(i, carry):
      rows = pl.ds(pl.multiple_of(i * 128, 128), 128)
      xr = xt_v[:, rows].astype(F32)
      t1 = xr * st_v[1, 0:1, rows] - st_v[2, 0:1, rows]
      out_v[:, rows] = (xr + (col_v[2] * t1 + col_v[3])).astype(BF16)
      pltpu.make_async_copy(out_v.at[:, rows], out_hbm.at[0, :, rows], out_sems.at[0]).start()
      return carry

    lax.fori_loop(0, S // 128, base_out, 0)

    bits = pltpu.bitcast(st_v[0], jnp.int32)
    hi = lax.shift_right_arithmetic(bits, 16)
    mono = jnp.where(hi < 0, hi ^ 0x7FFF, hi) + 32768
    col = lax.broadcasted_iota(jnp.int32, (8, S), 1)
    key_bits = 0x20000000 | lax.shift_left(mono, 11) | (2047 - col)
    key = pltpu.bitcast(key_bits, F32)
    lane = lax.broadcasted_iota(jnp.int32, (D // 2, 128), 1)
    xsel = jnp.zeros((D // 2, 128), U32)
    tiles, lanes = [], []
    for t in range(TOPC):
      best = jnp.max(key, axis=1, keepdims=True)
      key = jnp.where(key == best, 0.0, key)
      bi = 2047 - (pltpu.bitcast(best, jnp.int32) & 2047)
      idx = bi[0, 0]
      tiles.append(lax.shift_right_logical(idx, 7))
      lanes.append(idx & 127)
      tile = pl.ds(pl.multiple_of(tiles[t] * 128, 128), 128)
      xcol = pltpu.roll(pltpu.bitcast(xt_v[:, tile], U32), (t - lanes[t]) & 127, 1)
      xsel = jnp.where(lane == t, xcol, xsel)
    lasts = []
    for t in range(TOPC - 1):
      ok = tiles[t + 1] != tiles[t]
      for t2 in range(t + 2, TOPC):
        ok = jnp.logical_and(ok, tiles[t2] != tiles[t])
      lasts.append(ok)

    xs = pltpu.bitcast(xsel, BF16).astype(F32).T[0:8, :]
    modb = modb_v[...]
    sb, cb, gb = modb[:, D:2 * D], modb[:, 2 * D:3 * D], modb[:, 3 * D:4 * D]
    cen = xs - jnp.sum(xs, axis=1, keepdims=True) * (1.0 / D)
    var = jnp.sum(cen * cen, axis=1, keepdims=True) * (1.0 / D)
    hs = _rb(cen * lax.rsqrt(var + EPS) * cb + sb)
    r_sel = _rb(jnp.sum(hs * wr, axis=1, keepdims=True))
    xsb = jnp.concatenate([hs, jnp.zeros((8, D), F32)], axis=0).astype(BF16)
    gate = _rb(jnp.dot(xsb, wg_v[...], preferred_element_type=F32))
    gate = _rb(gate * jax.nn.sigmoid(gate))
    up = _rb(jnp.dot(xsb, wu_v[...], preferred_element_type=F32))
    gu = (gate * up).astype(BF16)
    wd = pltpu.bitcast(pltpu.bitcast(wdt_v[...].T, U32), BF16)
    y = jnp.dot(gu, wd, preferred_element_type=F32)[0:8, :]
    y = _rb(y) * _rb(jax.nn.sigmoid(r_sel))
    res = xs + gb * (hs + y)
    res = jnp.concatenate([res, jnp.zeros((128 - 8, D), F32)], axis=0).T
    res_p = pltpu.bitcast(res.astype(BF16), U32)

    pltpu.make_async_copy(out_v, out_hbm.at[0], out_sems.at[0]).wait()

    def patch_cp(t):
      tile = pl.ds(pl.multiple_of(tiles[t] * 128, 128), 128)
      return pltpu.make_async_copy(out_v.at[:, tile], out_hbm.at[0, :, tile], patch_sems.at[t])

    for t in range(TOPC):
      tile = pl.ds(pl.multiple_of(tiles[t] * 128, 128), 128)
      cur = pltpu.bitcast(out_v[:, tile], U32)
      new = jnp.where(lane == lanes[t], pltpu.roll(res_p, (lanes[t] - t) & 127, 1), cur)
      out_v[:, tile] = pltpu.bitcast(new, BF16)
      if t == TOPC - 1:
        patch_cp(t).start()
      else:
        pl.when(lasts[t])(lambda t=t: patch_cp(t).start())
    for t in range(TOPC - 1):
      pl.when(lasts[t])(lambda t=t: patch_cp(t).wait())
    patch_cp(TOPC - 1).wait()


@jax.jit
def pallas_adaLN_cond__gqa_block_cached__moe_arch_mod__prompt_kernel(
    A_x: jax.Array,
    A_k_cache: jax.Array,
    A_v_cache: jax.Array,
    A_wq: jax.Array,
    A_wo: jax.Array,
    B_x: jax.Array,
    B_w_r: jax.Array,
    B_w_gate: jax.Array,
    B_w_up: jax.Array,
    B_w_down: jax.Array,
    c: jax.Array,
    w_mod: jax.Array,
):
  del B_x
  any_spec = pl.BlockSpec(memory_space=pl.ANY)
  vmem = pltpu.VMEM
  scratch = [
      vmem((D, S), BF16),
      vmem((HQ, S, DH), BF16),
      vmem((HQ, S, DH), BF16),
      vmem((2, S, DH), BF16),
      vmem((2, S, DH), BF16),
      vmem((D, HQ * DH), BF16),
      vmem((D, HQ * DH), BF16),
      vmem((D,), BF16),
      vmem((D, FF), BF16),
      vmem((D, FF), BF16),
      vmem((D, FF), BF16),
      vmem((1, D), BF16),
      vmem((D, 6 * D), BF16),
      vmem((8, 4 * D), F32),
      vmem((4, D, 128), F32),
      vmem((3, 8, S), F32),
      vmem((D, S), BF16),
      pltpu.SemaphoreType.DMA((10,)),
      pltpu.SemaphoreType.DMA((2, 2)),
      pltpu.SemaphoreType.DMA((NWC,)),
      pltpu.SemaphoreType.DMA((1,)),
      pltpu.SemaphoreType.DMA((TOPC,)),
  ]
  out_t = pl.pallas_call(
      _kernel,
      in_specs=[any_spec] * 11,
      out_specs=any_spec,
      out_shape=jax.ShapeDtypeStruct((1, D, S), BF16),
      scratch_shapes=scratch,
      compiler_params=pltpu.CompilerParams(vmem_limit_bytes=110 * 1024 * 1024),
      name="adaln_gqa_mod_fused",
  )(jnp.swapaxes(A_x, 1, 2), A_k_cache, A_v_cache, A_wq, A_wo.T, B_w_r, B_w_gate,
    B_w_up, B_w_down.T, c, w_mod)
  return jnp.swapaxes(out_t, 1, 2)
```

```python
import contextlib
import math

import jax
import jax.numpy as jnp
from jax import lax
import jax.experimental.pallas as pl
import jax.experimental.pallas.tpu as pltpu

F32 = jnp.float32
BF16 = jnp.bfloat16
U32 = jnp.uint32
NT_DIMS = (((1,), (1,)), ((), ()))

S = 2048
D = 576
HQ = 32
HKV = 16
DH = 128
FF = 4608
TOPC = 8
EPS = 1e-5
Q_BLOCKS = ((512, 512, 512, 512), (512, 512, 384, 384, 256))
BM = 256
NBM = S // BM
WQ_CHUNKS = ((0, 512), (512, 1024), (1536, 1536), (3072, 1024))
NWC = len(WQ_CHUNKS)
QSCALE = (DH ** -0.5) * math.log2(math.e)
PROFILE = False


def _scope(name):
  return jax.named_scope(name) if PROFILE else contextlib.nullcontext()


def _rb(x):
  return x.astype(BF16).astype(F32)


def _ln_mod_t(x, scale1, shift):
  inv_d = 1.0 / D
  cen = x - jnp.sum(x, axis=0, keepdims=True) * inv_d
  var = jnp.sum(cen * cen, axis=0, keepdims=True) * inv_d
  return cen * lax.rsqrt(var + EPS) * scale1 + shift


def _rep(a, n):
  return jnp.concatenate([a] * (n // 128), axis=1) if n > 128 else a


def _cols(row):
  return jnp.broadcast_to(row, (128, row.shape[1])).T


def _kernel(xt_hbm, k_hbm, v_hbm, wq_hbm, wot_hbm, wr_hbm, wg_hbm, wu_hbm, wdt_hbm,
            c_hbm, wm_hbm, out_hbm,
            xt_v, x1_v, q_v, o_v, k_v, v_v, wq_v, wot_v, wr_v, wg_v, wu_v, wdt_v,
            c_v, wm_v, modb_v, col_v, st_v, out_v,
            sems, kv_sems, wq_sems, out_sems, patch_sems):

  def cp(src, dst, i):
    return pltpu.make_async_copy(src, dst, sems.at[i])

  c_cp = cp(c_hbm, c_v, 0)
  wm_a_cp = cp(wm_hbm.at[:, pl.ds(0, 2 * D)], wm_v.at[:, pl.ds(0, 2 * D)], 1)
  x_a_cp = cp(xt_hbm.at[0, :, pl.ds(0, 2 * BM)], xt_v.at[:, pl.ds(0, 2 * BM)], 2)
  x_b_cp = cp(xt_hbm.at[0, :, pl.ds(2 * BM, S - 2 * BM)], xt_v.at[:, pl.ds(2 * BM, S - 2 * BM)], 3)
  wm_b_cp = cp(wm_hbm.at[:, pl.ds(2 * D, 4 * D)], wm_v.at[:, pl.ds(2 * D, 4 * D)], 4)
  wo_cp = cp(wot_hbm, wot_v, 5)
  wr_cp = cp(wr_hbm, wr_v, 6)
  wg_cp = cp(wg_hbm, wg_v, 7)
  wu_cp = cp(wu_hbm, wu_v, 8)
  wd_cp = cp(wdt_hbm, wdt_v, 9)
  wq_cps = [pltpu.make_async_copy(wq_hbm.at[:, pl.ds(c0, n)], wq_v.at[:, pl.ds(c0, n)], wq_sems.at[i])
            for i, (c0, n) in enumerate(WQ_CHUNKS)]

  def kv_cp(g, slot):
    return (pltpu.make_async_copy(k_hbm.at[0, g], k_v.at[slot], kv_sems.at[0, slot]),
            pltpu.make_async_copy(v_hbm.at[0, g], v_v.at[slot], kv_sems.at[1, slot]))

  c_cp.start()
  x_a_cp.start()
  wm_a_cp.start()
  wq_cps[0].start()

  def ln_stats(x):
    cen = x - jnp.sum(x, axis=0, keepdims=True) * (1.0 / D)
    var = jnp.sum(cen * cen, axis=0, keepdims=True) * (1.0 / D)
    return cen * lax.rsqrt(var + EPS)

  with _scope("prologue"):
    c_cp.wait()
    cf = c_v[...].astype(F32)
    sc = _rb(cf * jax.nn.sigmoid(cf))
    sc16 = jnp.broadcast_to(sc, (16, D)).astype(BF16)
    x_a_cp.wait()
    xn01 = ln_stats(xt_v[:, pl.ds(0, 2 * BM)].astype(F32))
    wm_a_cp.wait()
    wq_cps[1].start()
    mod_a = jnp.dot(sc16, wm_v[:, pl.ds(0, 2 * D)], preferred_element_type=F32)
    mod_a = _cols(_rb(mod_a[0:1, :]))
    sa1 = mod_a[0:D] * QSCALE
    ca11 = _rb(1.0 + mod_a[D:2 * D]) * QSCALE

  def ln_apply(xn):
    n = xn.shape[1]
    return (xn * _rep(ca11, n) + _rep(sa1, n)).T.astype(BF16)

  def qproj(h, tok0, n, col0, ncol):
    q = jnp.dot(h, wq_v[:, pl.ds(col0, ncol)], preferred_element_type=F32)
    q = q.astype(BF16)
    for hl in range(ncol // DH):
      q_v[col0 // DH + hl, pl.ds(tok0, n), :] = q[:, hl * DH:(hl + 1) * DH]

  with _scope("qproj"):
    h01 = ln_apply(xn01)
    for ci, d in enumerate(wq_cps):
      d.wait()
      if ci + 2 < NWC:
        wq_cps[ci + 2].start()
      if ci == NWC - 3:
        x_b_cp.start()
      if ci == NWC - 1:
        x_b_cp.wait()
        for d2 in kv_cp(0, 0):
          d2.start()
        for d2 in (wm_b_cp, wr_cp, wo_cp, wg_cp, wu_cp, wd_cp):
          d2.start()
      qproj(h01, 0, 2 * BM, *WQ_CHUNKS[ci])
    tok0 = 2 * BM
    for n in (384,384,256,256,256):
      h = ln_apply(ln_stats(xt_v[:, pl.ds(tok0, n)].astype(F32)))
      qproj(h, tok0, n, 0, HQ * DH)
      tok0 += n

  def group(g, carry):
    slot = g % 2
    nxt = kv_cp(jnp.minimum(g + 1, HKV - 1), 1 - slot)
    k = k_v[slot]
    v = v_v[slot]
    for a, blocks in enumerate(Q_BLOCKS):
      hd = g * (HQ // HKV) + a
      row0 = 0
      for bq in blocks:
        rows = pl.ds(row0, bq)
        s = lax.dot_general(q_v[hd, rows, :], k, NT_DIMS, preferred_element_type=F32)
        m = jnp.max(s, axis=1, keepdims=True)
        p = jnp.exp2(s - m).astype(BF16)
        l = jnp.sum(p.astype(F32), axis=1, keepdims=True)
        o = jnp.dot(p, v, preferred_element_type=F32)
        o_v[hd, rows, :] = (o * pltpu.reciprocal(l, approx=True)).astype(BF16)
        if a == 0 and row0 == 0:
          for d in nxt:
            d.start()
        row0 += bq
    for d in nxt:
      d.wait()
    return carry

  with _scope("attn"):
    for d in kv_cp(0, 0):
      d.wait()
    lax.fori_loop(0, HKV, group, 0)

  with _scope("oproj"):
    wo_cp.wait()
    wm_b_cp.wait()
    wr_cp.wait()
    mod_b = jnp.dot(sc16, wm_v[:, pl.ds(2 * D, 4 * D)], preferred_element_type=F32)
    lane_b = lax.broadcasted_iota(jnp.int32, (1, 4 * D), 1)
    mod_b = _rb(mod_b[0:1, :])
    mod_b = jnp.where((lane_b >= 2 * D) & (lane_b < 3 * D), _rb(1.0 + mod_b), mod_b)
    modb_v[...] = jnp.broadcast_to(mod_b, (8, 4 * D))
    mod_c = _cols(mod_b)
    wr = wr_v[...].astype(F32).reshape(1, D)
    ga1, sb1, cb1, gb1 = mod_c[0:D], mod_c[D:2 * D], mod_c[2 * D:3 * D], mod_c[3 * D:4 * D]
    wr1 = _cols(wr)
    uw1 = cb1 * wr1
    for t, a in enumerate((ga1, uw1, gb1 * cb1, gb1 * sb1)):
      col_v[t] = a
    usum = _rep(jnp.sum(uw1, axis=0, keepdims=True), BM)
    rconst = _rep(jnp.sum(sb1 * wr1, axis=0, keepdims=True), BM)

    for i in range(NBM):
      rows = pl.ds(i * BM, BM)
      o_cat = jnp.concatenate([o_v[hd, rows, :] for hd in range(HQ)], axis=1)
      att = lax.dot_general(wot_v[...], o_cat, NT_DIMS, preferred_element_type=F32)
      x1 = xt_v[:, rows].astype(F32) + _rep(col_v[0], BM) * att
      x1_v[:, rows] = x1
      xt_v[:, rows] = x1.astype(BF16)
      c0 = x1[0:1, :]
      d0 = x1 - c0
      m0 = jnp.sum(d0, axis=0, keepdims=True) * (1.0 / D)
      var = jnp.sum(d0 * d0, axis=0, keepdims=True) * (1.0 / D) - m0 * m0
      rstd = lax.rsqrt(var + EPS)
      r = (jnp.sum(d0 * _rep(col_v[1], BM), axis=0, keepdims=True) - m0 * usum) * rstd + rconst
      st_v[0, :, rows] = jnp.broadcast_to(_rb(r), (8, BM))
      st_v[1, :, rows] = jnp.broadcast_to(rstd, (8, BM))
      st_v[2, :, rows] = jnp.broadcast_to((c0 + m0) * rstd, (8, BM))

  with _scope("tail"):
    wg_cp.wait()
    wu_cp.wait()
    wd_cp.wait()

    def base_out(i, carry):
      rows = pl.ds(pl.multiple_of(i * 128, 128), 128)
      xr = x1_v[:, rows]
      t1 = xr * st_v[1, 0:1, rows] - st_v[2, 0:1, rows]
      out_v[:, rows] = (xr + (col_v[2] * t1 + col_v[3])).astype(BF16)
      pltpu.make_async_copy(out_v.at[:, rows], out_hbm.at[0, :, rows], out_sems.at[0]).start()
      return carry

    lax.fori_loop(0, S // 128, base_out, 0)

    bits = pltpu.bitcast(st_v[0], jnp.int32)
    hi = lax.shift_right_arithmetic(bits, 16)
    mono = jnp.where(hi < 0, hi ^ 0x7FFF, hi) + 32768
    col = lax.broadcasted_iota(jnp.int32, (8, S), 1)
    key_bits = 0x20000000 | lax.shift_left(mono, 11) | (2047 - col)
    key = pltpu.bitcast(key_bits, F32)
    lane = lax.broadcasted_iota(jnp.int32, (D // 2, 128), 1)
    xsel = jnp.zeros((D // 2, 128), U32)
    tiles, lanes = [], []
    for t in range(TOPC):
      best = jnp.max(key, axis=1, keepdims=True)
      key = jnp.where(key == best, 0.0, key)
      bi = 2047 - (pltpu.bitcast(best, jnp.int32) & 2047)
      idx = bi[0, 0]
      tiles.append(lax.shift_right_logical(idx, 7))
      lanes.append(idx & 127)
      tile = pl.ds(pl.multiple_of(tiles[t] * 128, 128), 128)
      xcol = pltpu.roll(pltpu.bitcast(xt_v[:, tile], U32), (t - lanes[t]) & 127, 1)
      xsel = jnp.where(lane == t, xcol, xsel)
    lasts = []
    for t in range(TOPC - 1):
      ok = tiles[t + 1] != tiles[t]
      for t2 in range(t + 2, TOPC):
        ok = jnp.logical_and(ok, tiles[t2] != tiles[t])
      lasts.append(ok)

    xs = pltpu.bitcast(xsel, BF16).astype(F32).T[0:8, :]
    modb = modb_v[...]
    sb, cb, gb = modb[:, D:2 * D], modb[:, 2 * D:3 * D], modb[:, 3 * D:4 * D]
    cen = xs - jnp.sum(xs, axis=1, keepdims=True) * (1.0 / D)
    var = jnp.sum(cen * cen, axis=1, keepdims=True) * (1.0 / D)
    hs = _rb(cen * lax.rsqrt(var + EPS) * cb + sb)
    r_sel = _rb(jnp.sum(hs * wr, axis=1, keepdims=True))
    xsb = jnp.concatenate([hs, jnp.zeros((8, D), F32)], axis=0).astype(BF16)
    gate = _rb(jnp.dot(xsb, wg_v[...], preferred_element_type=F32))
    gate = _rb(gate * jax.nn.sigmoid(gate))
    up = _rb(jnp.dot(xsb, wu_v[...], preferred_element_type=F32))
    gu = (gate * up).astype(BF16)
    wd = pltpu.bitcast(pltpu.bitcast(wdt_v[...].T, U32), BF16)
    y = jnp.dot(gu, wd, preferred_element_type=F32)[0:8, :]
    y = _rb(y) * _rb(jax.nn.sigmoid(r_sel))
    res = xs + gb * (hs + y)
    resb = res.astype(BF16).astype(F32)

    pltpu.make_async_copy(out_v, out_hbm.at[0], out_sems.at[0]).wait()

    def patch_cp(t):
      tile = pl.ds(pl.multiple_of(tiles[t] * 128, 128), 128)
      return pltpu.make_async_copy(out_v.at[:, tile], out_hbm.at[0, :, tile], patch_sems.at[t])

    for t in range(TOPC):
      tile = pl.ds(pl.multiple_of(tiles[t] * 128, 128), 128)
      cur = pltpu.bitcast(out_v[:, tile], U32)
      colb = jnp.broadcast_to(resb[t:t + 1, :], (128, D)).astype(BF16).T
      new = jnp.where(lane == lanes[t], pltpu.bitcast(colb, U32), cur)
      out_v[:, tile] = pltpu.bitcast(new, BF16)
      if t == TOPC - 1:
        patch_cp(t).start()
      else:
        pl.when(lasts[t])(lambda t=t: patch_cp(t).start())
    for t in range(TOPC - 1):
      pl.when(lasts[t])(lambda t=t: patch_cp(t).wait())
    patch_cp(TOPC - 1).wait()


@jax.jit
def pallas_adaLN_cond__gqa_block_cached__moe_arch_mod__prompt_kernel(
    A_x: jax.Array,
    A_k_cache: jax.Array,
    A_v_cache: jax.Array,
    A_wq: jax.Array,
    A_wo: jax.Array,
    B_x: jax.Array,
    B_w_r: jax.Array,
    B_w_gate: jax.Array,
    B_w_up: jax.Array,
    B_w_down: jax.Array,
    c: jax.Array,
    w_mod: jax.Array,
):
  del B_x
  any_spec = pl.BlockSpec(memory_space=pl.ANY)
  vmem = pltpu.VMEM
  scratch = [
      vmem((D, S), BF16),
      vmem((D, S), F32),
      vmem((HQ, S, DH), BF16),
      vmem((HQ, S, DH), BF16),
      vmem((2, S, DH), BF16),
      vmem((2, S, DH), BF16),
      vmem((D, HQ * DH), BF16),
      vmem((D, HQ * DH), BF16),
      vmem((D,), BF16),
      vmem((D, FF), BF16),
      vmem((D, FF), BF16),
      vmem((D, FF), BF16),
      vmem((1, D), BF16),
      vmem((D, 6 * D), BF16),
      vmem((8, 4 * D), F32),
      vmem((4, D, 128), F32),
      vmem((3, 8, S), F32),
      vmem((D, S), BF16),
      pltpu.SemaphoreType.DMA((10,)),
      pltpu.SemaphoreType.DMA((2, 2)),
      pltpu.SemaphoreType.DMA((NWC,)),
      pltpu.SemaphoreType.DMA((1,)),
      pltpu.SemaphoreType.DMA((TOPC,)),
  ]
  out_t = pl.pallas_call(
      _kernel,
      in_specs=[any_spec] * 11,
      out_specs=any_spec,
      out_shape=jax.ShapeDtypeStruct((1, D, S), BF16),
      scratch_shapes=scratch,
      compiler_params=pltpu.CompilerParams(vmem_limit_bytes=110 * 1024 * 1024),
      name="adaln_gqa_mod_fused",
  )(jnp.swapaxes(A_x, 1, 2), A_k_cache, A_v_cache, A_wq, A_wo.T, B_w_r, B_w_gate,
    B_w_up, B_w_down.T, c, w_mod)
  return jnp.swapaxes(out_t, 1, 2)
```

```python
import contextlib
import math

import jax
import jax.numpy as jnp
from jax import lax
import jax.experimental.pallas as pl
import jax.experimental.pallas.tpu as pltpu

F32 = jnp.float32
BF16 = jnp.bfloat16
U32 = jnp.uint32
NT_DIMS = (((1,), (1,)), ((), ()))

S = 2048
D = 576
HQ = 32
HKV = 16
DH = 128
FF = 4608
TOPC = 8
EPS = 1e-5
Q_BLOCKS = ((512, 512, 512, 512), (512, 512, 384, 384, 256))
BM = 256
NBM = S // BM
WQ_CHUNKS = ((0, 512), (512, 1024), (1536, 1536), (3072, 1024))
NWC = len(WQ_CHUNKS)
QSCALE = (DH ** -0.5) * math.log2(math.e)
PROFILE = False


def _scope(name):
  return jax.named_scope(name) if PROFILE else contextlib.nullcontext()


def _rb(x):
  return x.astype(BF16).astype(F32)


def _ln_mod_t(x, scale1, shift):
  inv_d = 1.0 / D
  cen = x - jnp.sum(x, axis=0, keepdims=True) * inv_d
  var = jnp.sum(cen * cen, axis=0, keepdims=True) * inv_d
  return cen * lax.rsqrt(var + EPS) * scale1 + shift


def _rep(a, n):
  return jnp.concatenate([a] * (n // 128), axis=1) if n > 128 else a


def _cols(row):
  return jnp.broadcast_to(row, (128, row.shape[1])).T


def _kernel(xt_hbm, k_hbm, v_hbm, wq_hbm, wot_hbm, wr_hbm, wg_hbm, wu_hbm, wdt_hbm,
            c_hbm, wm_hbm, out_hbm,
            xt_v, x1_v, q_v, o_v, k_v, v_v, wq_v, wot_v, wr_v, wg_v, wu_v, wdt_v,
            c_v, wm_v, modb_v, col_v, st_v, out_v,
            sems, kv_sems, wq_sems, out_sems, patch_sems):

  def cp(src, dst, i):
    return pltpu.make_async_copy(src, dst, sems.at[i])

  c_cp = cp(c_hbm, c_v, 0)
  wm_a_cp = cp(wm_hbm.at[:, pl.ds(0, 2 * D)], wm_v.at[:, pl.ds(0, 2 * D)], 1)
  x_a_cp = cp(xt_hbm.at[0, :, pl.ds(0, 2 * BM)], xt_v.at[:, pl.ds(0, 2 * BM)], 2)
  x_b_cp = cp(xt_hbm.at[0, :, pl.ds(2 * BM, S - 2 * BM)], xt_v.at[:, pl.ds(2 * BM, S - 2 * BM)], 3)
  wm_b_cp = cp(wm_hbm.at[:, pl.ds(2 * D, 4 * D)], wm_v.at[:, pl.ds(2 * D, 4 * D)], 4)
  wo_cp = cp(wot_hbm, wot_v, 5)
  wr_cp = cp(wr_hbm, wr_v, 6)
  wg_cp = cp(wg_hbm, wg_v, 7)
  wu_cp = cp(wu_hbm, wu_v, 8)
  wd_cp = cp(wdt_hbm, wdt_v, 9)
  wq_cps = [pltpu.make_async_copy(wq_hbm.at[:, pl.ds(c0, n)], wq_v.at[:, pl.ds(c0, n)], wq_sems.at[i])
            for i, (c0, n) in enumerate(WQ_CHUNKS)]

  def kv_cp(g, slot):
    return (pltpu.make_async_copy(k_hbm.at[0, g], k_v.at[slot], kv_sems.at[0, slot]),
            pltpu.make_async_copy(v_hbm.at[0, g], v_v.at[slot], kv_sems.at[1, slot]))

  c_cp.start()
  x_a_cp.start()
  wm_a_cp.start()
  wq_cps[0].start()

  def ln_stats(x):
    cen = x - jnp.sum(x, axis=0, keepdims=True) * (1.0 / D)
    var = jnp.sum(cen * cen, axis=0, keepdims=True) * (1.0 / D)
    return cen * lax.rsqrt(var + EPS)

  with _scope("prologue"):
    c_cp.wait()
    cf = c_v[...].astype(F32)
    sc = _rb(cf * jax.nn.sigmoid(cf))
    sc16 = jnp.broadcast_to(sc, (16, D)).astype(BF16)
    x_a_cp.wait()
    xn01 = ln_stats(xt_v[:, pl.ds(0, 2 * BM)].astype(F32))
    wm_a_cp.wait()
    wq_cps[1].start()
    mod_a = jnp.dot(sc16, wm_v[:, pl.ds(0, 2 * D)], preferred_element_type=F32)
    mod_a = _cols(_rb(mod_a[0:1, :]))
    sa1 = mod_a[0:D] * QSCALE
    ca11 = _rb(1.0 + mod_a[D:2 * D]) * QSCALE

  def ln_apply(xn):
    n = xn.shape[1]
    return (xn * _rep(ca11, n) + _rep(sa1, n)).T.astype(BF16)

  def qproj(h, tok0, n, col0, ncol):
    q = jnp.dot(h, wq_v[:, pl.ds(col0, ncol)], preferred_element_type=F32)
    q = q.astype(BF16)
    for hl in range(ncol // DH):
      q_v[col0 // DH + hl, pl.ds(tok0, n), :] = q[:, hl * DH:(hl + 1) * DH]

  with _scope("qproj"):
    h01 = ln_apply(xn01)
    for ci, d in enumerate(wq_cps):
      d.wait()
      if ci + 2 < NWC:
        wq_cps[ci + 2].start()
      if ci == NWC - 3:
        x_b_cp.start()
      if ci == NWC - 1:
        x_b_cp.wait()
        for d2 in kv_cp(0, 0):
          d2.start()
        for d2 in (wm_b_cp, wr_cp, wo_cp, wg_cp, wu_cp, wd_cp):
          d2.start()
      qproj(h01, 0, 2 * BM, *WQ_CHUNKS[ci])
    tok0 = 2 * BM
    for n in (384, 384, 256, 256, 256):
      h = ln_apply(ln_stats(xt_v[:, pl.ds(tok0, n)].astype(F32)))
      qproj(h, tok0, n, 0, HQ * DH)
      tok0 += n

  def group(g, carry):
    slot = g % 2
    nxt = kv_cp(jnp.minimum(g + 1, HKV - 1), 1 - slot)
    k = k_v[slot]
    v = v_v[slot]
    for a, blocks in enumerate(Q_BLOCKS):
      hd = g * (HQ // HKV) + a
      row0 = 0
      for bq in blocks:
        rows = pl.ds(row0, bq)
        s = lax.dot_general(q_v[hd, rows, :], k, NT_DIMS, preferred_element_type=F32)
        m = jnp.max(s, axis=1, keepdims=True)
        p = jnp.exp2(s - m).astype(BF16)
        l = jnp.sum(p.astype(F32), axis=1, keepdims=True)
        o = jnp.dot(p, v, preferred_element_type=F32)
        o_v[hd, rows, :] = (o * pltpu.reciprocal(l, approx=True)).astype(BF16)
        if a == 0 and row0 == 0:
          for d in nxt:
            d.start()
        row0 += bq
    for d in nxt:
      d.wait()
    return carry

  with _scope("attn"):
    for d in kv_cp(0, 0):
      d.wait()
    lax.fori_loop(0, HKV, group, 0)

  with _scope("oproj"):
    wo_cp.wait()
    wm_b_cp.wait()
    wr_cp.wait()
    mod_b = jnp.dot(sc16, wm_v[:, pl.ds(2 * D, 4 * D)], preferred_element_type=F32)
    lane_b = lax.broadcasted_iota(jnp.int32, (1, 4 * D), 1)
    mod_b = _rb(mod_b[0:1, :])
    mod_b = jnp.where((lane_b >= 2 * D) & (lane_b < 3 * D), _rb(1.0 + mod_b), mod_b)
    modb_v[...] = jnp.broadcast_to(mod_b, (8, 4 * D))
    mod_c = _cols(mod_b)
    wr = wr_v[...].astype(F32).reshape(1, D)
    ga1, sb1, cb1, gb1 = mod_c[0:D], mod_c[D:2 * D], mod_c[2 * D:3 * D], mod_c[3 * D:4 * D]
    wr1 = _cols(wr)
    uw1 = cb1 * wr1
    for t, a in enumerate((ga1, uw1, gb1 * cb1, gb1 * sb1)):
      col_v[t] = a
    usum = _rep(jnp.sum(uw1, axis=0, keepdims=True), BM)
    rconst = _rep(jnp.sum(sb1 * wr1, axis=0, keepdims=True), BM)

    for i in range(NBM):
      rows = pl.ds(i * BM, BM)
      o_cat = jnp.concatenate([o_v[hd, rows, :] for hd in range(HQ)], axis=1)
      att = lax.dot_general(wot_v[...], o_cat, NT_DIMS, preferred_element_type=F32)
      x1 = xt_v[:, rows].astype(F32) + _rep(col_v[0], BM) * att
      x1_v[:, rows] = x1
      xt_v[:, rows] = x1.astype(BF16)
      c0 = x1[0:1, :]
      d0 = x1 - c0
      m0 = jnp.sum(d0, axis=0, keepdims=True) * (1.0 / D)
      var = jnp.sum(d0 * d0, axis=0, keepdims=True) * (1.0 / D) - m0 * m0
      rstd = lax.rsqrt(var + EPS)
      r = (jnp.sum(d0 * _rep(col_v[1], BM), axis=0, keepdims=True) - m0 * usum) * rstd + rconst
      st_v[0, :, rows] = jnp.broadcast_to(_rb(r), (8, BM))
      st_v[1, :, rows] = jnp.broadcast_to(rstd, (8, BM))
      st_v[2, :, rows] = jnp.broadcast_to((c0 + m0) * rstd, (8, BM))

  with _scope("tail"):
    wg_cp.wait()
    wu_cp.wait()
    wd_cp.wait()

    def base_out(i, carry):
      for u in range(2):
        rows = pl.ds(pl.multiple_of(i * 256 + u * 128, 128), 128)
        xr = x1_v[:, rows]
        t1 = xr * st_v[1, 0:1, rows] - st_v[2, 0:1, rows]
        out_v[:, rows] = (xr + (col_v[2] * t1 + col_v[3])).astype(BF16)
      rows = pl.ds(pl.multiple_of(i * 256, 256), 256)
      pltpu.make_async_copy(out_v.at[:, rows], out_hbm.at[0, :, rows], out_sems.at[0]).start()
      return carry

    lax.fori_loop(0, S // 256, base_out, 0)

    bits = pltpu.bitcast(st_v[0], jnp.int32)
    hi = lax.shift_right_arithmetic(bits, 16)
    mono = jnp.where(hi < 0, hi ^ 0x7FFF, hi) + 32768
    col = lax.broadcasted_iota(jnp.int32, (8, S), 1)
    key_bits = 0x20000000 | lax.shift_left(mono, 11) | (2047 - col)
    key = pltpu.bitcast(key_bits, F32)
    lane = lax.broadcasted_iota(jnp.int32, (D // 2, 128), 1)
    xsel = jnp.zeros((D // 2, 128), U32)
    tiles, lanes = [], []
    for t in range(TOPC):
      best = jnp.max(key, axis=1, keepdims=True)
      key = jnp.where(key == best, 0.0, key)
      bi = 2047 - (pltpu.bitcast(best, jnp.int32) & 2047)
      idx = bi[0, 0]
      tiles.append(lax.shift_right_logical(idx, 7))
      lanes.append(idx & 127)
      tile = pl.ds(pl.multiple_of(tiles[t] * 128, 128), 128)
      xcol = pltpu.roll(pltpu.bitcast(xt_v[:, tile], U32), (t - lanes[t]) & 127, 1)
      xsel = jnp.where(lane == t, xcol, xsel)
    lasts = []
    for t in range(TOPC - 1):
      ok = tiles[t + 1] != tiles[t]
      for t2 in range(t + 2, TOPC):
        ok = jnp.logical_and(ok, tiles[t2] != tiles[t])
      lasts.append(ok)

    xs = pltpu.bitcast(xsel, BF16).astype(F32).T[0:8, :]
    modb = modb_v[...]
    sb, cb, gb = modb[:, D:2 * D], modb[:, 2 * D:3 * D], modb[:, 3 * D:4 * D]
    cen = xs - jnp.sum(xs, axis=1, keepdims=True) * (1.0 / D)
    var = jnp.sum(cen * cen, axis=1, keepdims=True) * (1.0 / D)
    hs = _rb(cen * lax.rsqrt(var + EPS) * cb + sb)
    r_sel = _rb(jnp.sum(hs * wr, axis=1, keepdims=True))
    xsb = jnp.concatenate([hs, jnp.zeros((8, D), F32)], axis=0).astype(BF16)
    gate = _rb(jnp.dot(xsb, wg_v[...], preferred_element_type=F32))
    gate = _rb(gate * jax.nn.sigmoid(gate))
    up = _rb(jnp.dot(xsb, wu_v[...], preferred_element_type=F32))
    gu = (gate * up).astype(BF16)
    wd = pltpu.bitcast(pltpu.bitcast(wdt_v[...].T, U32), BF16)
    y = jnp.dot(gu, wd, preferred_element_type=F32)[0:8, :]
    y = _rb(y) * _rb(jax.nn.sigmoid(r_sel))
    res = xs + gb * (hs + y)
    resb = res.astype(BF16).astype(F32)

    pltpu.make_async_copy(out_v, out_hbm.at[0], out_sems.at[0]).wait()

    def patch_cp(t):
      tile = pl.ds(pl.multiple_of(tiles[t] * 128, 128), 128)
      return pltpu.make_async_copy(out_v.at[:, tile], out_hbm.at[0, :, tile], patch_sems.at[t])

    for t in range(TOPC):
      tile = pl.ds(pl.multiple_of(tiles[t] * 128, 128), 128)
      cur = pltpu.bitcast(out_v[:, tile], U32)
      colb = jnp.broadcast_to(resb[t:t + 1, :], (128, D)).astype(BF16).T
      new = jnp.where(lane == lanes[t], pltpu.bitcast(colb, U32), cur)
      out_v[:, tile] = pltpu.bitcast(new, BF16)
      if t == TOPC - 1:
        patch_cp(t).start()
      else:
        pl.when(lasts[t])(lambda t=t: patch_cp(t).start())
    for t in range(TOPC - 1):
      pl.when(lasts[t])(lambda t=t: patch_cp(t).wait())
    patch_cp(TOPC - 1).wait()


@jax.jit
def pallas_adaLN_cond__gqa_block_cached__moe_arch_mod__prompt_kernel(
    A_x: jax.Array,
    A_k_cache: jax.Array,
    A_v_cache: jax.Array,
    A_wq: jax.Array,
    A_wo: jax.Array,
    B_x: jax.Array,
    B_w_r: jax.Array,
    B_w_gate: jax.Array,
    B_w_up: jax.Array,
    B_w_down: jax.Array,
    c: jax.Array,
    w_mod: jax.Array,
):
  del B_x
  any_spec = pl.BlockSpec(memory_space=pl.ANY)
  vmem = pltpu.VMEM
  scratch = [
      vmem((D, S), BF16),
      vmem((D, S), F32),
      vmem((HQ, S, DH), BF16),
      vmem((HQ, S, DH), BF16),
      vmem((2, S, DH), BF16),
      vmem((2, S, DH), BF16),
      vmem((D, HQ * DH), BF16),
      vmem((D, HQ * DH), BF16),
      vmem((D,), BF16),
      vmem((D, FF), BF16),
      vmem((D, FF), BF16),
      vmem((D, FF), BF16),
      vmem((1, D), BF16),
      vmem((D, 6 * D), BF16),
      vmem((8, 4 * D), F32),
      vmem((4, D, 128), F32),
      vmem((3, 8, S), F32),
      vmem((D, S), BF16),
      pltpu.SemaphoreType.DMA((10,)),
      pltpu.SemaphoreType.DMA((2, 2)),
      pltpu.SemaphoreType.DMA((NWC,)),
      pltpu.SemaphoreType.DMA((1,)),
      pltpu.SemaphoreType.DMA((TOPC,)),
  ]
  out_t = pl.pallas_call(
      _kernel,
      in_specs=[any_spec] * 11,
      out_specs=any_spec,
      out_shape=jax.ShapeDtypeStruct((1, D, S), BF16),
      scratch_shapes=scratch,
      compiler_params=pltpu.CompilerParams(vmem_limit_bytes=110 * 1024 * 1024),
      name="adaln_gqa_mod_fused",
  )(jnp.swapaxes(A_x, 1, 2), A_k_cache, A_v_cache, A_wq, A_wo.T, B_w_r, B_w_gate,
    B_w_up, B_w_down.T, c, w_mod)
  return jnp.swapaxes(out_t, 1, 2)
```
